```python
import os as _os
_os.environ.setdefault("JAX_PLATFORMS", "cpu")
import jax
import jax.numpy as jnp

def _softmax(x, axis=-1):
    return jax.nn.softmax(x, axis=axis)
def _gelu(x):
    return jax.nn.gelu(x, approximate=True)
def _silu(x):
    return jax.nn.silu(x)
def _sigmoid(x):
    return jax.nn.sigmoid(x)
def _layernorm(x, axis=-1, eps=1e-5):
    m = jnp.mean(x, axis=axis, keepdims=True)
    v = jnp.var(x, axis=axis, keepdims=True)
    return (x - m) / jnp.sqrt(v + eps)
def _scatter_add(tgt, idx, src, axis=0):
    return tgt.at[idx].add(src)
def _segment_sum(src, seg, n):
    return jax.ops.segment_sum(src, seg, n)
class _Rng:
    def __init__(self, key):
        self._k = key
    def _next(self):
        self._k, sub = jax.random.split(self._k)
        return sub
    def normal(self, shape):
        return jax.random.normal(self._next(), shape, dtype=jnp.bfloat16)
    def randint(self, lo, hi, shape):
        return jax.random.randint(self._next(), shape, lo, hi, dtype=jnp.int32)
    def uniform(self, shape, lo=0.0, hi=1.0):
        return jax.random.uniform(self._next(), shape, jnp.bfloat16, lo, hi)
    def permutation(self, n):
        return jax.random.permutation(self._next(), n)


kernel_name = 'sequential_preLN__softmax_full_mha__dense_activation_squared_relu__prompt'

def setup_inputs():
    _rng = _Rng(jax.random.key(int.from_bytes(__import__("os").urandom(4), "little")))
    _w = (lambda a: (lambda t: t.astype(jnp.bfloat16) if jnp.issubdtype(t.dtype, jnp.floating) else t)(jnp.asarray(a)))
    def _A_setup():
        B, S, D = 1, 2048, 448
        return {
            "x": _w((lambda *s: _rng.normal(s) * 0.05)(B, S, D)),
            "wqkv": _w((lambda *s: _rng.normal(s) * 0.05)(D, 3 * D)),
            "wo": _w((lambda *s: _rng.normal(s) * 0.05)(D, D)),
        }
    _A_in = _A_setup()

    def _B_setup():
        B, S, D, F = 1, 2048, 448, 1792
        return {
            "x": _w((lambda *s: _rng.normal(s) * 0.05)(B, S, D)),
            "w1": _w((lambda *s: _rng.normal(s) * 0.05)(D, F)),
            "b1": _w((lambda *s: _rng.normal(s) * 0.05)(F)),
            "w2": _w((lambda *s: _rng.normal(s) * 0.05)(F, D)),
            "b2": _w((lambda *s: _rng.normal(s) * 0.05)(D)),
        }
    _B_in = _B_setup()

    return {
        "A_x": _A_in["x"],
        "A_wqkv": _A_in["wqkv"],
        "A_wo": _A_in["wo"],
        "B_x": _B_in["x"],
        "B_w1": _B_in["w1"],
        "B_b1": _B_in["b1"],
        "B_w2": _B_in["w2"],
        "B_b2": _B_in["b2"],
    }

def reference(A_x, A_wqkv, A_wo, B_x, B_w1, B_b1, B_w2, B_b2):
    def _A_ref(x, wqkv, wo):
        B, S, D = x.shape
        H = 16; Dh = D // H
        qkv = (lambda x, *d: x.transpose(*d))((x @ wqkv).reshape(B, S, 3, H, Dh), 2, 0, 3, 1, 4)
        q, k, v = qkv[0], qkv[1], qkv[2]
        scale = Dh ** -0.5
        scores = jnp.einsum("bhqd,bhkd->bhqk", q, k) * scale
        p = _softmax(scores, axis=-1)
        o = jnp.einsum("bhqk,bhkd->bhqd", p, v)
        return (lambda x, *d: x.transpose(*d))(o, 0, 2, 1, 3).reshape(B, S, D) @ wo

    def _B_ref(x, w1, b1, w2, b2):
        h = jnp.einsum("bsd,df->bsf", x, w1) + b1
        zero = jnp.zeros_like(h)
        r = jnp.where(h > zero, h, zero)
        h = r * r
        out = jnp.einsum("bsf,fd->bsd", h, w2) + b2
        return out

    x = A_x
    h = x + _A_ref(_layernorm(x, axis=-1), A_wqkv, A_wo)
    h2 = h + _B_ref(_layernorm(h, axis=-1), B_w1, B_b1, B_w2, B_b2)
    return h2
```

```python
import functools
import math

import jax
import jax.numpy as jnp
from jax import lax
import jax.experimental.pallas as pl
import jax.experimental.pallas.tpu as pltpu

S, D, H, DH, F = 2048, 448, 16, 28, 1792
BQ = 512
NQ = S // BQ
KC = 128
NK = S // KC
HP = 32
EPS = 1e-5
QSCALE = DH ** -0.5 * math.log2(math.e)
bf16, f32 = jnp.bfloat16, jnp.float32


def _dot(a, b):
    return jnp.dot(a, b, preferred_element_type=f32)


def _layernorm_t(x):
    mean = jnp.sum(x, axis=0, keepdims=True) * (1.0 / D)
    xc = x - mean
    var = jnp.sum(xc * xc, axis=0, keepdims=True) * (1.0 / D)
    return xc * lax.rsqrt(var + EPS)


def _head_windows(y, fill):
    n = y.shape[1]
    low = lax.broadcasted_iota(jnp.int32, (8, n), 0) < 4
    out = []
    for p in range(2):
        r = 56 * p
        mid = y[r + 24:r + 32]
        out.append(jnp.concatenate([y[r:r + 24], jnp.where(low, mid, fill)], axis=0))
        out.append(jnp.concatenate([jnp.where(low, fill, mid), y[r + 32:r + 56]], axis=0))
    return out


def _kernel(x_hbm, wqkv_hbm, wo_hbm, w1_hbm, b1_hbm, w2t_hbm, b2_hbm, out_hbm,
            x_v, wqkv_v, wo_v, w1_v, b1_v, w2t_v, b2_v,
            wqkvt, wot, w1t, b2t, q_s, k_s, v_s, s_a, s_b, o_s, out_v,
            in_sems, out_sems, *, cfg):
    delta = cfg["delta"]
    unroll = cfg["unroll"]

    def x_copy(j):
        return pltpu.make_async_copy(x_hbm.at[:, pl.ds(j * BQ, BQ)], x_v.at[j], in_sems.at[j])

    w_copies = [pltpu.make_async_copy(src, dst, in_sems.at[NQ + i]) for i, (src, dst) in enumerate(
        [(wqkv_hbm, wqkv_v), (wo_hbm, wo_v), (w1_hbm, w1_v), (b1_hbm, b1_v), (w2t_hbm, w2t_v), (b2_hbm, b2_v)])]

    x_copy(0).start()
    w_copies[0].start()
    for j in range(1, NQ):
        x_copy(j).start()
    for c in w_copies[1:]:
        c.start()

    w_copies[0].wait()
    wqkvt[...] = wqkv_v[...].T

    def project(j, t):
        lanes = pl.ds(t * 128, 128)
        xn = _layernorm_t(x_v[j, :, lanes].astype(f32)).astype(bf16)
        for g in range(4):
            kt = _dot(wqkvt[pl.ds(D + 112 * g, 112), :], xn)
            kt = jnp.concatenate(_head_windows(kt, 0.0), axis=0).astype(bf16)
            k_s[g, j * (BQ // KC) + t] = kt.T
        for g in range(4):
            qt = _dot(wqkvt[pl.ds(112 * g, 112), :], xn) * QSCALE
            for i, w in enumerate(_head_windows(qt, 0.0)):
                q_s[j, 4 * g + i, :, lanes] = w.astype(bf16)
        for g in range(4):
            vt = _dot(wqkvt[pl.ds(2 * D + 112 * g, 112), :], xn)
            for i, w in enumerate(_head_windows(vt, 1.0)):
                v_s[4 * g + i, j * (BQ // KC) + t] = w.astype(bf16)

    def phase1(j, carry):
        x_copy(j).wait()
        for t in range(BQ // 128):
            project(j, t)
        return carry

    lax.fori_loop(0, NQ, phase1, 0)

    sbuf = (s_a, s_b)

    def qk_chunk(u, pos, c, par):
        q = q_s[u // H, u % H]
        zero = jnp.zeros((HP, BQ), bf16)
        qt = jnp.concatenate([q if i == pos else zero for i in range(4)], axis=0)
        s = _dot(k_s[(u % H) // 4, c], qt)
        sbuf[par][c] = s
        return jnp.max(s.reshape(KC // 8, 8, BQ), axis=0)

    def pv_chunk(u, m, c, par):
        p = jnp.exp2(sbuf[par][c] - m).astype(bf16)
        return _dot(v_s[u % H, c], p)

    def finish_quad(u0, accs):
        low = lax.broadcasted_iota(jnp.int32, (8, BQ), 0) < 4
        rows = []
        for p in range(2):
            a, b = accs[2 * p], accs[2 * p + 1]
            a = a * (1.0 / a[HP - 1:HP])
            b = b * (1.0 / b[0:1])
            rows += [a[:24], jnp.where(low, a[24:], b[:8]), b[8:]]
        o_s[u0 // H, (u0 % H) // 4] = jnp.concatenate(rows, axis=0).astype(bf16)

    def run_units(u0, n, carry, last=False):
        m, mx = carry
        accs = []
        for r in range(n):
            acc = None
            for c in range(NK):
                o = pv_chunk(u0 + r, m, c, r % 2)
                acc = o if acc is None else acc + o
                du, cq = 1 + (c + delta) // NK, (c + delta) % NK
                if cq == 0:
                    m_next = jnp.max(mx, axis=0, keepdims=True)
                if last and r + du >= n:
                    continue
                t = qk_chunk(u0 + r + du, (r + du) % 4, cq, (r + du) % 2)
                mx = t if cq == 0 else jnp.maximum(mx, t)
            m = m_next
            accs.append(acc)
            if r % 4 == 3:
                finish_quad(u0 + r - 3, accs)
                accs = []
        return m, mx

    for c in w_copies[1:]:
        c.wait()

    mx = None
    for c in range(NK):
        t = qk_chunk(0, 0, c, 0)
        mx = t if c == 0 else jnp.maximum(mx, t)
    m = jnp.max(mx, axis=0, keepdims=True)
    for c in range(delta):
        t = qk_chunk(1, 1, c, 1)
        mx = t if c == 0 else jnp.maximum(mx, t)

    wot[...] = wo_v[...].T
    row = lax.broadcasted_iota(jnp.int32, (64, F), 0)
    tail = jnp.where(row == 0, b1_v[...].astype(f32).reshape(1, F), 0.0).astype(bf16)
    w1t[...] = jnp.concatenate([w1_v[...], tail], axis=0).T
    b2t[...] = jnp.broadcast_to(b2_v[...].astype(f32).reshape(1, D), (128, D)).T

    n_tail = 4
    n_loop = (H * NQ - n_tail) // unroll
    assert n_loop * unroll + n_tail == H * NQ
    carry = lax.fori_loop(0, n_loop, lambda i, cr: run_units(i * unroll, unroll, cr), (m, mx))
    run_units(H * NQ - n_tail, n_tail, carry, last=True)

    def out_copy(j):
        return pltpu.make_async_copy(out_v.at[j], out_hbm.at[:, pl.ds(j * BQ, BQ)], out_sems.at[j])

    TW = cfg["tw"]

    def phase3(j, carry):
        hs = []
        for t in range(BQ // TW):
            lanes = pl.ds(t * TW, TW)
            o = jnp.concatenate([o_s[j, g, :, lanes] for g in range(4)], axis=0)
            hs.append(x_v[j, :, lanes].astype(f32) + _dot(wot[...], o))
        acts = []
        for t in range(BQ // TW):
            hn = _layernorm_t(hs[t]).astype(bf16)
            hn = jnp.concatenate([hn, jnp.ones((64, TW), bf16)], axis=0)
            u = jnp.maximum(_dot(w1t[...], hn), 0.0)
            acts.append((u * u).astype(bf16))
        for t in range(BQ // TW):
            lanes = pl.ds(t * TW, TW)
            bias = jnp.concatenate([b2t[...]] * (TW // 128), axis=1)
            out_v[j, :, lanes] = (hs[t] + bias + _dot(w2t_v[...], acts[t])).astype(bf16)
        out_copy(j).start()
        return carry

    lax.fori_loop(0, NQ, phase3, 0)
    for j in range(NQ):
        out_copy(j).wait()


DEFAULT = dict(delta=2, unroll=12, tw=256)


@jax.jit
def pallas_sequential_preLN__softmax_full_mha__dense_activation_squared_relu__prompt_kernel(
    A_x: jax.Array,
    A_wqkv: jax.Array,
    A_wo: jax.Array,
    B_x: jax.Array,
    B_w1: jax.Array,
    B_b1: jax.Array,
    B_w2: jax.Array,
    B_b2: jax.Array,
):
    cfg = DEFAULT
    del B_x
    any_spec = pl.BlockSpec(memory_space=pl.ANY)
    out_t = pl.pallas_call(
        functools.partial(_kernel, cfg=cfg),
        out_shape=jax.ShapeDtypeStruct((D, S), bf16),
        in_specs=[any_spec] * 7,
        out_specs=any_spec,
        scratch_shapes=[
            pltpu.VMEM((NQ, D, BQ), bf16),
            pltpu.VMEM((D, 3 * D), bf16),
            pltpu.VMEM((D, D), bf16),
            pltpu.VMEM((D, F), bf16),
            pltpu.VMEM((F,), bf16),
            pltpu.VMEM((D, F), bf16),
            pltpu.VMEM((D,), bf16),
            pltpu.VMEM((3 * D, D), bf16),
            pltpu.VMEM((D, D), bf16),
            pltpu.VMEM((F, 512), bf16),
            pltpu.VMEM((D, 128), f32),
            pltpu.VMEM((NQ, H, HP, BQ), bf16),
            pltpu.VMEM((4, NK, KC, 128), bf16),
            pltpu.VMEM((H, NK, HP, KC), bf16),
            pltpu.VMEM((NK, KC, BQ), f32),
            pltpu.VMEM((NK, KC, BQ), f32),
            pltpu.VMEM((NQ, 4, 112, BQ), bf16),
            pltpu.VMEM((NQ, D, BQ), bf16),
            pltpu.SemaphoreType.DMA((NQ + 6,)),
            pltpu.SemaphoreType.DMA((NQ,)),
        ],
        compiler_params=pltpu.CompilerParams(vmem_limit_bytes=100 * 2**20),
        name="fused_block",
    )(A_x.reshape(S, D).T, A_wqkv, A_wo, B_w1, B_b1, B_w2.T, B_b2)
    return out_t.T.reshape(1, S, D)
```

```python
import functools
import math

import jax
import jax.numpy as jnp
from jax import lax
import jax.experimental.pallas as pl
import jax.experimental.pallas.tpu as pltpu

S, D, H, DH, F = 2048, 448, 16, 28, 1792
BQ = 512
NQ = S // BQ
KC = 128
NK = S // KC
HP = 32
NP = H // 2
HD = D // 2
EPS = 1e-5
QSCALE = DH ** -0.5 * math.log2(math.e)
SUM_LO, SUM_HI = 2.0 ** -20, 2.0 ** 100
bf16, f32, u32 = jnp.bfloat16, jnp.float32, jnp.uint32

SV0 = 8
Q0 = SV0 + 32
DATA = Q0 + 2 * NQ * 8

ORDER = (1, 3, 2, 4, 0, 6, 5)


def _dot(a, b):
    return jnp.dot(a, b, preferred_element_type=f32)


def _pad_rows(x, n, value=0.0):
    return jnp.concatenate([x, jnp.full((n - x.shape[0], x.shape[1]), value, x.dtype)], axis=0)


def _tile(t):
    return pl.ds(128 * t, 128)


def _words(x):
    return pltpu.bitcast(x, u32).reshape(x.shape[0] // 16, 8, 128)


def _halves(w):
    return pltpu.bitcast(w.reshape(w.shape[0] * 8, 128), bf16)


def _head_windows(y, fill_a, fill_b):
    low = lax.broadcasted_iota(jnp.int32, (8, y.shape[1]), 0) < 4
    return (jnp.concatenate([y[:24], jnp.where(low, y[24:32], fill_a)], axis=0),
            jnp.concatenate([jnp.where(low, fill_b, y[24:32]), y[32:]], axis=0))


def _weight_term(i, quad):
    a, sign, b = (((0, 0), 1, (1, 1)), ((1, 0), 1, (1, 1)), ((0, 0), 0, None), ((1, 1), 0, None),
                  ((0, 0), 1, (0, 1)), ((1, 0), -1, (0, 0)), ((0, 1), -1, (1, 1)))[i]
    return quad(*a) if sign == 0 else quad(*a) + quad(*b) if sign > 0 else quad(*a) - quad(*b)


def _input_terms(top, bottom):
    n = top.shape[1] // 2
    b11, b12, b21, b22 = top[:, :n], top[:, n:], bottom[:, :n], bottom[:, n:]
    return [b11 + b22, b11, b12 - b22, b21 - b11, b22, b11 + b12, b21 + b22]


def _combine(m):
    return (jnp.concatenate([m[3] - m[4] + m[0] + m[6], m[2] + m[4]], axis=1),
            jnp.concatenate([m[1] + m[3], m[2] - m[1] + m[0] + m[5]], axis=1))


def _gate(ref, zero, value):
    if value is None:
        return
    if value.dtype == bf16:
        value = value.astype(f32)
    value = pltpu.bitcast(value, f32).astype(bf16) if ref.dtype == bf16 else pltpu.bitcast(value, ref.dtype)
    ref[(zero + ref.shape[0] - 1, *(0,) * (len(ref.shape) - 3), pl.ds(0, 8), _tile(0))] = value


class _Pacer:
    def __init__(self, zero, delay, slow):
        self.zero, self.delay, self.slow = zero, delay, slow
        self.tick, self.todo, self.done = 0, {}, {}

    def add(self, first, last, chores):
        for n, chore in enumerate(chores):
            self.todo.setdefault(self.tick + first + n * (last - first) // len(chores), []).append(chore)

    def wait(self, ticks, v):
        self.done.setdefault(self.tick + ticks, []).extend(v[-8:, l:l + 128] for l in range(0, v.shape[1], 128))

    def dot(self, w_ref, i, starts, rhs, cols=slice(None)):
        pieces = []
        for n, r in enumerate(starts):
            for k, v in enumerate(self.done.pop(self.tick + n, [])):
                v = v.astype(f32) if v.dtype == bf16 else pltpu.bitcast(v, f32)
                v = v.astype(bf16) if w_ref.dtype == bf16 else pltpu.bitcast(v, u32)
                w_ref[self.zero + w_ref.shape[0] - 1, pl.ds(8 * k, 8), _tile(0)] = v
            if w_ref.dtype == bf16:
                pieces.append(w_ref[i, pl.ds(r, 16), cols])
            else:
                pieces.append(pltpu.bitcast(w_ref[i, pl.ds(r // 2, 8), cols], bf16))
        y = _dot(jnp.concatenate(pieces, axis=0), rhs)
        for n in range(len(pieces)):
            for chore in self.todo.pop(self.tick + n, []):
                vs = chore(y[16 * n:16 * n + 8, :128])
                for k, v in enumerate(vs if isinstance(vs, tuple) else (vs,)):
                    self.wait(max(n + self.delay + k * self.slow, len(pieces)), v)
        self.tick += len(pieces)
        return y


def _norm_chores(src, j, zero, emit, report=None):
    st = {}

    def load(r, n):
        return src[j, pl.ds(r, n)].astype(f32)

    def total(r, clock):
        _gate(src, zero, clock)
        y = jnp.sum(load(r, 32).reshape(4, 8, BQ), axis=0)
        st["acc"] = y if r == 0 else st["acc"] + y
        return st["acc"]

    def spread(r, clock):
        _gate(src, zero, clock)
        if r == 0:
            st["mean"] = jnp.sum(st["acc"], axis=0, keepdims=True) * (1.0 / D)
        y = load(r, 32) - st["mean"]
        y = jnp.sum((y * y).reshape(4, 8, BQ), axis=0)
        st["acc"] = y if r == 0 else st["acc"] + y
        return st["acc"]

    def scale(r, clock):
        _gate(src, zero, clock)
        if r == 0:
            var = jnp.sum(st["acc"], axis=0, keepdims=True) * (1.0 / D)
            st["inv"] = lax.rsqrt(var + EPS)
            if report:
                report(var < jnp.inf)
        return emit(r, *((load(k + r, 8) - st["mean"]) * st["inv"] for k in (0, HD)))

    return ([functools.partial(f, r) for f in (total, spread) for r in range(0, D, 32)]
            + [functools.partial(scale, r) for r in range(0, HD, 8)])


def _kernel(x_hbm, wqkv_hbm, wo_hbm, w1_hbm, b1_hbm, w2t_hbm, b2_hbm, out_hbm,
            x_v, wqkv_v, wo_v, w1_v, w2t_v,
            wqk_s, wv_s, wo_s, w1_s, w2_s, b2_s, xn_s, m_s, keep, sums, acts, hn_s, h_s,
            pk, qw_s, qb_s, kt_s, kb, o_s, out_v, b1_s, b1_v, b2_v, zeros_s, in_sems, out_sems, *, cfg):
    noff, nseg, nb = cfg["noff"], cfg["nseg"], cfg["nb"]
    lag, L, W = cfg["lag"], cfg["L"], cfg["w"]
    seg_lo = [-(-(DH * s) // nseg) for s in range(nseg + 1)]
    seg_at = [sum(seg_lo[t + 1] - seg_lo[t] for t in range(s % nb, s, nb)) for s in range(nseg)]
    kb_at = [(s % nb, seg_at[s] + d - seg_lo[s]) for s in range(nseg) for d in range(seg_lo[s], seg_lo[s + 1])]
    on_vpu = [(noff * (c + 1)) // NK - (noff * c) // NK for c in range(NK)]
    nmm = [KC // 16 - n for n in on_vpu]
    T = HD // 16

    sources = [(x_hbm.at[:, pl.ds(j * BQ, BQ)], x_v.at[j]) for j in range(NQ)] + [
        (wqkv_hbm.at[:, pl.ds(2 * D, D)], wqkv_v.at[0, :, pl.ds(2 * D, D)]),
        (wqkv_hbm.at[:, pl.ds(0, 2 * D)], wqkv_v.at[0, :, pl.ds(0, 2 * D)]),
        (wo_hbm, wo_v.at[0]), (w1_hbm, w1_v.at[0]), (b1_hbm, b1_v), (w2t_hbm, w2t_v.at[0]), (b2_hbm, b2_v)]
    copies = [pltpu.make_async_copy(src, dst, in_sems.at[i]) for i, (src, dst) in enumerate(sources)]
    x_copies, wv_copy, mid_copies, late_copies = copies[:NQ], copies[NQ], copies[NQ + 1:NQ + 3], copies[NQ + 3:]

    wv_copy.start()
    x_copies[0].start()
    zeros_s[0] = 0
    zeros_s[1] = 0

    def k_slot(c, rr):
        return pk[(c + rr) % 2], DATA + c * 4 + rr // 2

    def v_slot(h, c, rr):
        return pk[(c + rr) % 2], DATA + (4 + h) * NK + c

    def norm_x(j, zero):
        def emit(r, top, bottom):
            xn_s[j][0, pl.ds(r, 8)] = top.astype(bf16)
            xn_s[j][0, pl.ds(HD + r, 8)] = bottom.astype(bf16)
            return xn_s[j][zero, pl.ds(r, 8), _tile(0)]
        return _norm_chores(x_v, j, zero, emit)

    def transpose_chores(dst, src, first, zero):
        def chore(k, c, clock):
            _gate(src, zero, clock)
            n = min(128, 2 * dst.shape[1] - c)
            y = src[0, pl.ds(256 * k, 256 - 64 * k), pl.ds(first + c, n)]
            y = pltpu.bitcast((_pad_rows(y, 256) if k else y).T, u32)
            dst[0, pl.ds(c // 2, n // 2), pl.ds(256 * k, 256)] = y
            return clock, y[:, :128]
        return [functools.partial(chore, k, c) for c in range(0, 2 * dst.shape[1], 128) for k in range(2)]

    def project_v(pace, j):
        for t in range(4 * (cfg['only'] != 2)):
            for r in range(0, D, HD):
                y = pace.dot(wv_s, zeros_s[1], range(r, r + HD, 16), _pad_rows(xn_s[j][pace.zero, :, _tile(t)], 512))
                for m in range(0, HD, 56):
                    for h, w in enumerate(_head_windows(y[m:m + 56], 1.0, 1.0)):
                        w = _words(w.astype(bf16))
                        for rr in range(2):
                            pool, at = v_slot(h, 4 * j + t, rr)
                            pool[(r + m) // 56, at] = w[rr]
                pace.wait(cfg["d1"], pool[pace.zero, at])

    def project_qk(pace, n, c):
        j, t = divmod(c, 4)
        starts = [k + 112 * n + r for r in range(0, 112, 16) for k in (0, D)]
        y = pace.dot(wqk_s, zeros_s[1], starts, _pad_rows(xn_s[j][pace.zero, :, _tile(t)], 512))
        qs, ks = (jnp.concatenate([y[r:r + 16] for r in range(k, HD, 32)], axis=0) for k in (0, 16))
        for m in range(2):
            g, qt, kt = 2 * n + m, qs[56 * m:56 * m + 56] * QSCALE, ks[56 * m:56 * m + 56]
            shift = [-jnp.sum(w, axis=0, keepdims=True) for w in _head_windows(qt * kt, 0.0, 0.0)]
            kw = _words(_pad_rows(jnp.concatenate(_head_windows(kt, 0.25, 0.25), axis=0), 128).astype(bf16).T)
            for rr in reversed(range(8)):
                pool, at = k_slot(c, rr)
                pool[g, at] = kw[7 - rr]
            for h, w in enumerate(_head_windows(qt, *shift)):
                w = _words(w.astype(bf16))
                qw_s[g, h * NQ + j, pl.ds(2 * t, 2)] = w
                if cfg['a2'] == 1:
                    for pool in pk:
                        pool[g, pl.ds(Q0 + (h * NQ + j) * 8 + 2 * t, 2)] = w
                q = _halves(w).astype(f32)
                for d in range(DH + 1):
                    row = (d + 4 * h) % HP
                    qb_s[g, h * NQ + j, t // W, d, t % W] = jnp.broadcast_to(q[row:row + 1], (8, 128))
            pace.wait(cfg["d2"] + 7 * m, qb_s[pace.zero, 0, 0, 0, 0])
            pace.wait(cfg["d3"] + 7 * m, kw[7])

    def gather_keys(g, e, zero):
        k = jnp.concatenate([k_slot(c, 7)[0][zero + g, k_slot(c, 7)[1]] for c in range(8 * e, 8 * e + 8)], axis=0)
        kt_s[g, e] = y = pltpu.bitcast(k, bf16).T[:2 * HP].astype(f32)
        return y

    def spread_keys(g, h, e, d):
        y = jnp.broadcast_to(kt_s[g, e, pl.ds(h * (HP + 4) + d, 1)], (128, 128)).T
        kb[h][kb_at[d][0]][kb_at[d][1], pl.ds(8 * e, 8)] = y.reshape(8, 2, 8, 128)
        return y

    wv_copy.wait()
    x_copies[1].start()
    for chore in transpose_chores(wv_s, wqkv_v, 2 * D, 0):
        chore(None)
    x_copies[0].wait()
    for c in x_copies[2:] + mid_copies:
        c.start()
    for chore in norm_x(0, zeros_s[0]):
        chore(None)
    x_copies[1].wait()
    pace = _Pacer(zeros_s[0], cfg["delay"], cfg["slow"])
    pace.add(0, 7 * T, norm_x(1, pace.zero))
    project_v(pace, 0)
    for c in x_copies[2:] + mid_copies:
        c.wait()
    for c in late_copies:
        c.start()
    pace = _Pacer(zeros_s[0], cfg["delay"], cfg["slow"])
    zero = pace.zero

    def spread_chore(e, d, clock):
        _gate(kt_s, zero, clock)
        return clock, spread_keys(0, 0, e, d)

    pace.add(0, 12 * T, transpose_chores(wqk_s, wqkv_v, 0, zero) + transpose_chores(wo_s, wo_v, 0, zero))
    for j in (1, 2):
        pace.add(0, 6 * T, norm_x(j + 1, zero))
        project_v(pace, j)
    for n in range(4 * (cfg['only'] != 2)):
        if n == 1:
            pace.add(3 * T, 4 * T, [lambda clock, e=e: (clock, gather_keys(0, e, zero)) for e in range(2)])
            pace.add(7 * T, 53 * T, [functools.partial(spread_chore, e, d) for e in range(2) for d in range(DH)])
        for c in range(NK):
            project_qk(pace, n, c)
    project_v(pace, 3)

    units = [(h, j) for h in range(2) for j in range(NQ)]
    nsteps = len(units) * NK
    ticks = []
    for i in range(nsteps + 1):
        if i < nsteps:
            ticks += [("k", i, r) for r in range(nmm[i % NK])]
        else:
            nhalf = 2 * len(ticks) + 4
            ticks += [("idle", 0, 1)] * nmm[0]
        if i >= 1:
            ticks += [("v", i - 1, r) for r in range(2)]
    segs = [(u, e, a, s) for u in range(len(units)) for e in range(NK) if on_vpu[e]
            for a in range(4 // W) for s in range(nseg)]
    sched, prod, qload, vload = {}, {}, {}, {}
    for i, sg in enumerate(segs):
        sched.setdefault(max((i * nhalf) // len(segs) + cfg["ph"], 0), []).append(sg)
    for h in range(2):
        for i in range(2 * DH):
            prod.setdefault((h * nhalf) // 2 + cfg["p0"] + i * cfg["ps"], []).append((1 - h, i // DH, i % DH))
    for t, x in enumerate(ticks):
        if x[2] == 0:
            if x[0] == "k":
                qload.setdefault(max(0, t - cfg["qa"]), []).append(x[1])
            else:
                vload.setdefault(t - cfg["va"], []).append(x[1])

    def attend(g, carry):
        zero = zeros_s[0]
        g_next = jnp.minimum(g + 1, NP - 1)
        for e in range(2):
            gather_keys(g_next, e, 0)
        res, lhs = [], []
        pend, where, vp, ps, qts = {}, {}, {}, {}, {}
        acc = vacc = None
        for tau, (kind, i, rr) in enumerate(ticks):
            u, c = divmod(i, NK)
            h, j = units[u]
            pool, at = k_slot(c, rr) if kind == "k" else v_slot(h, c, rr) if kind == "v" else (pk[tau % 2], None)
            for half in range(2):
                for (addr, v, key) in pend.pop(2 * tau + half, []):
                    pool[g, pl.ds(addr, v.shape[0])] = pltpu.bitcast(v, u32)
                    if key is not None:
                        where[key] = (pool, addr)
            for i2 in vload.get(tau, []):
                u2, c2 = divmod(i2, NK)
                if on_vpu[c2]:
                    parts = []
                    for a in range(4 // W):
                        p_, addr = where.pop((u2, c2, a))
                        parts.append(jnp.exp2(pltpu.bitcast(p_[g, pl.ds(addr, 2 * W)], f32)))
                    vp[i2] = [jnp.concatenate([parts[a][x * W + l] for a in range(4 // W) for l in range(W)], axis=1)
                              for x in range(2)]
            for i2 in qload.get(tau, []):
                h2, j2 = units[i2 // NK]
                if cfg['a2'] == 1:
                    w = _halves(pool[g, pl.ds(Q0 + (h2 * NQ + j2) * 8, 8)])
                elif cfg['a2'] == 2:
                    w = _halves(qw_s[g, h2 * NQ + j2])
                else:
                    _gate(qw_s, zero, res[2 * tau - L] if 0 <= 2 * tau - L < len(res) else None)
                    w = _halves(qw_s[g, h2 * NQ + j2])
                q = jnp.concatenate([w[HP * l:HP * l + HP] for l in range(4)], axis=1)
                qts[i2] = jnp.concatenate([q if x == h2 else jnp.zeros(q.shape, bf16) for x in range(4)], axis=0)
            if at is not None:
                lhs.append(pltpu.bitcast(pool[g, at], bf16))
            for half in range(2):
                now = 2 * tau + half
                clock = res[now - L] if 0 <= now - L < len(res) else None
                for (u2, e, a, s) in sched.get(now, []):
                    kpool = kb[units[u2][0]][s % nb]
                    nd = seg_lo[s + 1] - seg_lo[s]
                    _gate(kpool, zero, clock)
                    kv = kpool[pl.ds(seg_at[s], nd), e]
                    qv = qb_s[g, u2, a, pl.ds(seg_lo[s], nd)]
                    t = kv[:, :, None] * qv[:, None]
                    for d in range(nd):
                        vacc = t[d] if seg_lo[s] + d == 0 else vacc + t[d]
                    if s == nseg - 1:
                        vacc = vacc + qb_s[g, u2, a, DH][None]
                        slot = SV0 + (e % 4) * 8 + a * 2 * W
                        pend.setdefault(now + lag, []).append((slot, vacc.reshape(2 * W, 8, 128), (u2, e, a)))
                    else:
                        pend.setdefault(now + lag, []).append((zero + (s % 2) * W, vacc[s % 2], None))
                for (h2, e, d) in prod.get(now, []):
                    _gate(kt_s, zero, clock)
                    spread_keys(g if h2 else g_next, h2, e, d)
            if kind == "k" and rr == nmm[c] - 1:
                sc = _dot(jnp.concatenate(lhs, axis=0), qts.pop(i))
                lhs = []
                p = jnp.exp2(sc)
                ps[i] = [p[16 * x:16 * x + 16] for x in reversed(range(nmm[c]))]
                res += [sc[8 * x:8 * x + 8, :128] for x in range(2 * nmm[c])]
            if kind == "v" and rr == 1:
                o = _dot(jnp.concatenate(lhs, axis=0), jnp.concatenate(vp.pop(i, []) + ps.pop(i), axis=0))
                lhs = []
                acc = o if c == 0 else acc + o
                if c == NK - 1:
                    for l in range(4):
                        o_s[4 * j + l, g, h] = acc[:, 128 * l:128 * l + 128]
                res += [o[8 * x:8 * x + 8, :128] for x in range(4)]
        return carry

    if cfg["only"] == 1:
        o_s[zeros_s[0], 0, 0, pl.ds(0, 8)] = sum(p[zeros_s[0], 0, 0] for p in kb[0])
    else:
        lax.fori_loop(0, NP, attend, 0)

    def attend_true_max(n, carry):
        g, h, t = n // 32, (n // 16) % 2, n % 16
        q = _halves(qw_s[g, h * NQ + t // 4, pl.ds(2 * (t % 4), 2)]).astype(f32)
        r = lax.broadcasted_iota(jnp.int32, (4 * HP, 128), 0) - h * (HP + 4)
        q = jnp.where((r >= 0) & (r < DH), jnp.concatenate([q] * 4, axis=0), 0.0).astype(bf16)
        k = [k_slot(c, rr) for c in range(NK) for rr in reversed(range(8))]
        sc = _dot(pltpu.bitcast(jnp.concatenate([pool[g, at] for pool, at in k], axis=0), bf16), q)
        p = jnp.exp2(sc - jnp.max(sc, axis=0, keepdims=True))
        v = [jnp.concatenate([pool[g, at] for pool, at in [v_slot(h, c, rr) for c in range(NK)]], axis=1)
             for rr in range(2)]
        o_s[t, g, h] = _dot(pltpu.bitcast(jnp.concatenate(v, axis=0), bf16), p.astype(bf16))
        return carry

    if cfg['only'] == 2:
        out_v[0, pl.ds(0, 32), pl.ds(0, 128)] = o_s[zeros_s[0], 0, 0].astype(bf16)
        pltpu.sync_copy(out_v.at[0], out_hbm.at[:, pl.ds(0, BQ)])
        return
    for c in late_copies:
        c.wait()

    def out_copy(j):
        return pltpu.make_async_copy(out_v.at[j], out_hbm.at[:, pl.ds(j * BQ, BQ)], out_sems.at[j])

    def finish(attempt):
        @pl.when(attempt == 1)
        def _():
            lax.fori_loop(0, H * S // 128, attend_true_max, 0)

        pace = _Pacer(zeros_s[0], cfg["delay"], cfg["slow"])
        zero = pace.zero
        flag = {"unsafe": jnp.zeros((8, 128), f32)}

        def report(safe):
            for l in range(0, safe.shape[1], 128):
                flag["unsafe"] = jnp.where(safe[:, l:l + 128], flag["unsafe"], 1.0)

        def heads(t):
            low = lax.broadcasted_iota(jnp.int32, (8, 128), 0) < 4
            rows = []
            for g in range(NP):
                a, b = o_s[t, g, 0], o_s[t, g, 1]
                total = jnp.where(low, b[:8], a[24:])
                report((total >= SUM_LO) & (total <= SUM_HI))
                inv = pltpu.reciprocal(total, full_range=False)
                a, b = a * inv[7:], b * inv[:1]
                rows += [a[:24], jnp.where(low, a[24:], b[:8]), b[8:]]
            return _pad_rows(jnp.concatenate(rows, axis=0), 512).astype(bf16)

        def norm_h(j, zero):
            def emit(r, top, bottom):
                for i, t in enumerate(_input_terms(top, bottom)):
                    hn_s[i, pl.ds(r, 8)] = t.astype(bf16)
                return hn_s[zero, pl.ds(r, 8), _tile(0)]
            return _norm_chores(h_s, j, zero, emit, report)

        def w1_chore(n, i, clock):
            _gate(w1_v, zero, clock)
            t = _weight_term(i, lambda m, k: w1_v[0, pl.ds(HD * k, HD), _tile(7 * m + n)].astype(f32))
            if i in (1, 4, 5, 6):
                t = jnp.concatenate([t, b1_s[:, _tile(n + (7 if i in (1, 5) else 0))] * (2.0 if i > 4 else 1.0)], axis=0)
            w1_s[i, pl.ds(64 * n, 64)] = pltpu.bitcast(_pad_rows(t, 256).astype(bf16).T, u32)
            return t[:HD], w1_s[zero + i, pl.ds(64 * n, 8), _tile(0)]

        b1_s[...] = jnp.where(lax.broadcasted_iota(jnp.int32, (8, F), 0) == 0, b1_v[...].astype(f32).reshape(1, F), 0.0)
        b2_s[...] = jnp.broadcast_to(b2_v[...].astype(f32).reshape(1, D), (128, D)).T
        pace.add(0, 30 * T, [functools.partial(w1_chore, n, i) for n in range(7) for i in range(7)])
        pace.add(10 * T, 31 * T, norm_h(0, zero))
        clock = None
        for t in range(NK):
            _gate(o_s, zero, clock)
            rhs = heads(t)
            for r in range(0, D, HD):
                y = pace.dot(wo_s, 0, range(r, r + HD, 16), rhs)
                at = (t // 4, pl.ds(r, HD), _tile(t % 4))
                h_s[at] = x_v[at].astype(f32) + y
                clock = y[:8] if r == 0 else clock

        def ffn(j, unsafe):
            flag["unsafe"] = unsafe
            pace = _Pacer(zeros_s[0], cfg["delay"], cfg["slow"])
            zero = pace.zero
            lo, size = (0, 256, 512, 640), (256, 256, 128, 256)

            def w2_chore(r, c, clock):
                _gate(w2t_v, zero, clock)
                n = min(256, F // 2 - c)
                quads = [[w2t_v[0, pl.ds(HD * m + r, 16), pl.ds(F // 2 * k + c, n)].astype(f32) for k in range(2)]
                         for m in range(2)]
                for i in range(7):
                    w2_s[i, pl.ds(r, 16), pl.ds(c, n)] = _weight_term(i, lambda m, k: quads[m][k]).astype(bf16)
                return w2_s[zero, pl.ds(r, 8), pl.ds(c, 128)]

            def act_chore(n, r, clock):
                _gate(m_s[n % 3], zero, clock)
                us = [jnp.maximum(u, 0.0) for u in _combine([m_s[n % 3][i, pl.ds(r, 8)] for i in range(7)])]
                for i, t in enumerate(_input_terms(*[u * u for u in us])):
                    acts[n // 3][i, pl.ds(lo[n] % 640 + r, 8)] = t.astype(bf16)
                return acts[n // 3][zero, pl.ds(lo[n] % 640 + r, 8), _tile(0)]

            pace.add(0, cfg["n3"] * T, [functools.partial(w2_chore, r, c) for r in range(0, HD, 16) for c in range(0, F // 2, 256)])
            for n, (first, last) in enumerate(((0, 104), (0, 100), (44, 92), (0, 104))):
                for i in ORDER:
                    m_s[n % 3][i, pl.ds(0, size[n])] = pace.dot(
                        w1_s, i, range(lo[n], lo[n] + size[n], 16), _pad_rows(hn_s[zero + i], 256, 1.0))
                pace.add(first, last, [functools.partial(act_chore, n, r) for r in range(0, size[n], 8)])

            def product(k, n, i):
                rhs = acts[n // 3][zero + i, pl.ds(lo[n] % 640, size[n])]
                return pace.dot(w2_s, zeros_s[1] + i, range(0, HD, 16), rhs, pl.ds(lo[n], size[n])) + sums[k][zero + i]

            def at(n, l):
                return j, pl.ds(HD * n, HD), pl.ds(256 * l, 256)

            def base(n, l):
                return h_s[at(n, l)] + jnp.concatenate([b2_s[pl.ds(HD * n, HD)]] * 2, axis=1)

            for i in ORDER:
                parts = [pl.ds(0, HD)] if i != ORDER[-1] else [pl.ds(0, HD // 2), pl.ds(HD // 2, HD // 2)]
                for k, rows in enumerate(parts):
                    sums[0][i, rows] = _dot(w2_s[zeros_s[1] + i, rows, pl.ds(lo[2], 128)],
                                            acts[0][zeros_s[k] + i, pl.ds(lo[2], 128)])
            for k in range(2):
                if k == 1:
                    pace.add(0, cfg["n5"] * T, norm_h(jnp.minimum(j + 1, NQ - 1), zero))
                for i in ORDER:
                    sums[1 - k][i] = product(k, k, i)
            keep[0][0] = product(0, 3, 1)
            keep[1][0] = y = product(0, 3, 3)
            out_v[at(1, 0)] = (y + keep[0][zero] + base(1, 0)).astype(bf16)
            keep[1][1] = y = product(0, 3, 2)
            keep[1][2] = y - keep[0][zero] + base(1, 1)
            y = product(0, 3, 4)
            out_v[at(0, 1)] = (y + keep[1][zero + 1] + base(0, 1)).astype(bf16)
            keep[0][1] = keep[1][zero] - y + base(0, 0)
            keep[0][2] = product(0, 3, 0)
            out_v[at(0, 0)] = (keep[0][zero + 1] + keep[0][zero + 2] + product(0, 3, 6)).astype(bf16)
            out_v[at(1, 1)] = (keep[1][zero + 2] + keep[0][zero + 2] + product(0, 3, 5)).astype(bf16)
            out_copy(j).start()
            return flag["unsafe"]

        unsafe = lax.fori_loop(0, NQ, ffn, flag["unsafe"])
        redo = (jnp.max(unsafe) > 0.0) & (attempt == 0)
        for j in range(NQ):
            out_copy(j).wait()
        return jnp.where(redo, 1, 2)

    lax.while_loop(lambda attempt: attempt < 2, finish, 0)


DEFAULT = dict(noff=16, w=2, lag=2, L=20, qa=4, va=2, nb=3, nseg=9, ps=18, p0=40, ph=1, only=0, a2=2,
               delay=16, slow=28, d1=14, d2=12, d3=32, n3=9, n5=9)


@jax.jit
def pallas_sequential_preLN__softmax_full_mha__dense_activation_squared_relu__prompt_kernel(
    A_x: jax.Array,
    A_wqkv: jax.Array,
    A_wo: jax.Array,
    B_x: jax.Array,
    B_w1: jax.Array,
    B_b1: jax.Array,
    B_w2: jax.Array,
    B_b2: jax.Array,
):
    cfg = DEFAULT
    del B_x
    any_spec = pl.BlockSpec(memory_space=pl.ANY)
    W, nb = cfg["w"], cfg["nb"]
    out_t = pl.pallas_call(
        functools.partial(_kernel, cfg=cfg),
        out_shape=jax.ShapeDtypeStruct((D, S), bf16),
        in_specs=[any_spec] * 7,
        out_specs=any_spec,
        scratch_shapes=[
            pltpu.VMEM((NQ + 1, D, BQ), bf16),
            pltpu.VMEM((2, D, 3 * D), bf16),
            pltpu.VMEM((2, D, D), bf16),
            pltpu.VMEM((2, D, F), bf16),
            pltpu.VMEM((2, D, F), bf16),
            pltpu.VMEM((2, D, 512), u32),
            pltpu.VMEM((2, HD, 512), u32),
            pltpu.VMEM((2, HD, 512), u32),
            pltpu.VMEM((8, F // 4, 256), u32),
            pltpu.VMEM((8, HD, F // 2), bf16),
            pltpu.VMEM((D, 128), f32),
            [pltpu.VMEM((2, D, BQ), bf16)] * NQ,
            [pltpu.VMEM((8, 256, 256), f32)] * 3,
            [pltpu.VMEM((3, HD, 256), f32)] * 2,
            [pltpu.VMEM((7, HD, 256), f32)] * 2,
            [pltpu.VMEM((7, n, 256), bf16) for n in (640, 256)],
            pltpu.VMEM((7, HD, 256), bf16),
            pltpu.VMEM((NQ + 1, D, BQ), f32),
            [pltpu.VMEM((NP, DATA + 6 * NK, 8, 128), u32)] * 2,
            pltpu.VMEM((NP + 1, 2 * NQ, 8, 8, 128), u32),
            pltpu.VMEM((NP, 2 * NQ, 4 // W, DH + 1, W, 8, 128), f32),
            pltpu.VMEM((NP + 1, 2, 2 * HP, 128), f32),
            [[pltpu.VMEM((-(-DH // nb) + 2, NK + 1, 2, 8, 128), f32)] * nb] * 2,
            pltpu.VMEM((NK + 1, NP, 2, HP, 128), f32),
            pltpu.VMEM((NQ, D, BQ), bf16),
            pltpu.VMEM((8, F), f32),
            pltpu.VMEM((F,), bf16),
            pltpu.VMEM((D,), bf16),
            pltpu.SMEM((2,), jnp.int32),
            pltpu.SemaphoreType.DMA((NQ + 7,)),
            pltpu.SemaphoreType.DMA((NQ,)),
        ],
        compiler_params=pltpu.CompilerParams(vmem_limit_bytes=110 * 2**20),
        name="fused_block",
    )(A_x.reshape(S, D).T, A_wqkv, A_wo, B_w1, B_b1, B_w2.T, B_b2)
    return out_t.T.reshape(1, S, D)
```

```python
import functools
import math

import jax
import jax.numpy as jnp
from jax import lax
import jax.experimental.pallas as pl
import jax.experimental.pallas.tpu as pltpu

S, D, H, DH, F = 2048, 448, 16, 28, 1792
BQ = 512
NQ = S // BQ
KC = 128
NK = S // KC
HP = 32
NP = H // 2
HD = D // 2
EPS = 1e-5
QSCALE = DH ** -0.5 * math.log2(math.e)
SUM_LO, SUM_HI = 2.0 ** -20, 2.0 ** 100
bf16, f32, u32 = jnp.bfloat16, jnp.float32, jnp.uint32

SCORES, PIECES = 8, 40

SEG_LO = [-(-(DH * s) // 9) for s in range(10)]
SEG_AT = [sum(SEG_LO[t + 1] - SEG_LO[t] for t in range(s % 3, s, 3)) for s in range(9)]
KEY_AT = [(s % 3, SEG_AT[s] + d - SEG_LO[s]) for s in range(9) for d in range(SEG_LO[s], SEG_LO[s + 1])]
ROW_OF = [[8 * k + r for r in range(8) for k in range(4) if 0 <= 8 * k + r - 4 * h < DH] for h in range(2)]

PASS_ROWS = ((384, 256), (0, 64), (128, 192), (384, 320), (256, 320))

ORDER = (1, 3, 2, 4, 0, 6, 5)
PART_LO, PART = (0, 256, 512, 640), (256, 256, 128, 256)
TICKS = HD // 16


def _dot(a, b):
    return jnp.dot(a, b, preferred_element_type=f32)


def _tile(t):
    return pl.ds(128 * t, 128)


def _pad_rows(x, n, value=0.0):
    return jnp.concatenate([x, jnp.full((n - x.shape[0], x.shape[1]), value, x.dtype)], axis=0)


def _words(x):
    return pltpu.bitcast(x, u32).reshape(x.shape[0] // 16, 8, 128)


def _halves(w):
    return pltpu.bitcast(w.reshape(w.shape[0] * 8, 128), bf16)


def _head_windows(y, fill):
    low = lax.broadcasted_iota(jnp.int32, (8, y.shape[1]), 0) < 4
    return (jnp.concatenate([y[:24], jnp.where(low, y[24:32], fill)], axis=0),
            jnp.concatenate([jnp.where(low, fill, y[24:32]), y[32:]], axis=0))


def _weight_term(i, quad):
    a, sign, b = (((0, 0), 1, (1, 1)), ((1, 0), 1, (1, 1)), ((0, 0), 0, None), ((1, 1), 0, None),
                  ((0, 0), 1, (0, 1)), ((1, 0), -1, (0, 0)), ((0, 1), -1, (1, 1)))[i]
    return quad(*a) if sign == 0 else quad(*a) + quad(*b) if sign > 0 else quad(*a) - quad(*b)


def _input_terms(b11, b12, b21, b22):
    return [b11 + b22, b11, b12 - b22, b21 - b11, b22, b11 + b12, b21 + b22]


def _retype(v, dtype):
    if v.dtype == dtype:
        return v
    if v.dtype != f32:
        v = v.astype(f32) if v.dtype == bf16 else pltpu.bitcast(v, f32)
    return v if dtype == f32 else v.astype(bf16) if dtype == bf16 else pltpu.bitcast(v, dtype)


def _gate(ref, zero, value, row=0):
    if value is not None:
        at = (zero + (ref.shape[0] - 1), *(0,) * (len(ref.shape) - 3), pl.ds(row, 8), _tile(0))
        ref[at] = _retype(value, ref.dtype)


class _Pacer:
    def __init__(self, zero, delay):
        self.zero, self.delay = zero, delay
        self.tick, self.todo, self.due = 0, {}, {}

    def add(self, first, last, chores):
        for n, chore in enumerate(chores):
            self.todo.setdefault(self.tick + first + n * (last - first) // len(chores), []).append(chore)

    def deadline(self, ticks, v):
        self.due.setdefault(self.tick + ticks, []).extend(v[-8:, l:l + 128] for l in range(0, v.shape[1], 128))

    def dots(self, w_ref, *jobs):
        pieces, ticks = [[] for _ in jobs], len(jobs[0][1])
        for n in range(ticks):
            for k, v in enumerate(self.due.pop(self.tick + n, [])):
                _gate(w_ref, self.zero, v, 8 * k)
            for got, (i, starts, cols, _) in zip(pieces, jobs):
                r = starts[n]
                got.append(w_ref[i, pl.ds(r, 16) if w_ref.dtype == bf16 else pl.ds(r // 2, 8), cols])
        lhs = [jnp.concatenate(got, axis=0) for got in pieces]
        ys = [_dot(a if a.dtype == bf16 else pltpu.bitcast(a, bf16), job[3]) for a, job in zip(lhs, jobs)]
        for n in range(ticks):
            for chore in self.todo.pop(self.tick + n, []):
                done = chore(ys[0][16 * n:16 * n + 8, :128])
                for k, v in enumerate(done if isinstance(done, tuple) else (done,)):
                    self.deadline(max(n + self.delay + 28 * k, ticks), v)
        self.tick += ticks
        return ys

    def dot_pair(self, w_ref, i, x):
        firsts = [range(r, r + 112, 16) for r in range(0, D, 112)]
        for k, first in enumerate(firsts):
            shared, y = self.dots(
                w_ref, (i, first, _tile(4), jnp.concatenate([x(256, 64, 0), x(320, 64, 1)], axis=0)),
                (i, first, pl.ds(128, 384), jnp.concatenate([x(0, 256, 0), x(384, 128, 0)], axis=0)))
            yield k, 0, shared + y
            if k == 0:
                late = shared
                continue
            rhs = [x(384, 128, 1), x(0, 128, 1), x(128, 128, 1)]
            part, y = self.dots(w_ref, (i, firsts[0], _tile(k - 1), rhs[k - 1]),
                                (i, first, pl.ds(0, 384), jnp.concatenate(rhs, axis=0)))
            late = late + part
            yield k, 1, shared + y
        yield 0, 1, late

    def close(self):
        assert not self.todo


def _norm_chores(src, j, cols, runs, zero, emit, report=None):
    step = 8 * BQ // cols.size
    st = {}

    def load(r, n):
        return src[j, pl.ds(r, n), cols].astype(f32)

    def total(r, clock):
        _gate(src, zero, clock)
        y = jnp.sum(load(r, 4 * step).reshape(-1, 8, cols.size), axis=0)
        st["acc"] = y if r == 0 else st["acc"] + y
        return st["acc"]

    def spread(r, clock):
        _gate(src, zero, clock)
        if r == 0:
            st["mean"] = jnp.sum(st["acc"], axis=0, keepdims=True) * (1.0 / D)
        y = load(r, 4 * step) - st["mean"]
        y = jnp.sum((y * y).reshape(-1, 8, cols.size), axis=0)
        st["acc"] = y if r == 0 else st["acc"] + y
        return st["acc"]

    def scale(r, n, clock):
        _gate(src, zero, clock)
        if r == 0:
            var = jnp.sum(st["acc"], axis=0, keepdims=True) * (1.0 / D)
            st["inv"] = lax.rsqrt(var + EPS)
            if report:
                report(var < jnp.inf)
        return emit(r, n, *((load(k, step) - st["mean"]) * st["inv"] for k in (r, r + n)))

    return ([functools.partial(f, r) for f in (total, spread) for r in range(0, D, 4 * step)]
            + [functools.partial(scale, r, n) for first, n in runs for r in range(first, first + n, step)])


def _kernel(x_hbm, wqkv_hbm, wo_hbm, w1_hbm, b1_hbm, w2t_hbm, b2_hbm, out_hbm,
            x_v, wqkv_v, wo_v, w1_v, w2t_v,
            wqk_s, wv_s, wo_s, w1_s, w2_s, b2_s, xn_s, raw_s, m_s, keep, sums, acts, hn_s, h_s,
            pools, qw_s, qb_s, kmean_s, kt_s, kb_s, tail_s, o_s, out_v,
            b1_s, b1_v, b2_v, zeros_s, in_sems, out_sem):
    waves = [[(wqkv_hbm.at[:, pl.ds(2 * D, D)], wqkv_v.at[0, :, pl.ds(2 * D, D)])]]
    waves += [[(x_hbm.at[:, pl.ds(j * BQ, BQ)], x_v.at[j]) for j in js] for js in ((0,), (1,), (2, 3))]
    waves += [[(wqkv_hbm.at[:, pl.ds(0, 2 * D)], wqkv_v.at[0, :, pl.ds(0, 2 * D)]), (wo_hbm, wo_v.at[0])],
              [(w1_hbm, w1_v.at[0]), (w2t_hbm, w2t_v.at[0])]]
    waves[2] += [(b1_hbm, b1_v), (b2_hbm, b2_v)]
    waves = [[pltpu.make_async_copy(src, dst, in_sems.at[i]) for src, dst in wave] for i, wave in enumerate(waves)]

    def land(i):
        for copy in waves[i]:
            copy.wait()
        for wave in waves[i + 2:i + 3]:
            for copy in wave:
                copy.start()
        return _Pacer(zeros_s[0], 16)

    for copy in waves[0] + waves[1]:
        copy.start()
    for z in range(4):
        zeros_s[z] = 0
    tail_s[...] = jnp.zeros(tail_s.shape, f32)

    def k_slot(c, rr):
        return pools[(c + rr) % 2], PIECES + c * 4 + rr // 2

    def v_slot(h, c, rr):
        return pools[(c + rr) % 2], h * NK + (PIECES + 4 * NK + c)

    def norm_x(p, zero):
        def emit(r, n, top, bottom):
            xn_s[p][zero, pl.ds(r, 16)] = top.astype(bf16)
            xn_s[p][zero, pl.ds(r + n, 16)] = bottom.astype(bf16)
            if 256 <= r < 320:
                diff = jnp.concatenate([bottom[:, :128] - bottom[:, 128:], top[:, 128:] - top[:, :128]], axis=1)
                xn_s[p][zero, pl.ds(D + r - 256, 16)] = diff.astype(bf16)
            return xn_s[p][0, pl.ds(r, 8), _tile(0)]
        return _norm_chores(x_v, p // 2, pl.ds(256 * (p % 2), 256), ((0, 128), (256, 64), (384, 32)), zero, emit)

    def transpose_chores(dst, src, first, zero, passes=PASS_ROWS):
        def chore(k, c, clock):
            _gate(src, zero, clock)
            n = min(256, 2 * dst.shape[1] - c)
            y = jnp.concatenate([src[0, pl.ds(r, 64), pl.ds(first + c, n)] for r in passes[k]], axis=0)
            y = pltpu.bitcast((y if y.shape[0] == 128 else _pad_rows(y, 128)).T, u32)
            dst[0, pl.ds(c // 2, n // 2), _tile(k)] = y
            return clock, y
        return [functools.partial(chore, k, c) for c in range(0, 2 * dst.shape[1], 256) for k in range(len(passes))]

    def project(pace, w_ref, p):
        return pace.dot_pair(w_ref, zeros_s[1], lambda r, n, t: xn_s[p][0, pl.ds(r, n), _tile(t)])

    def project_v(pace, p):
        for n, t, y in project(pace, wv_s, p):
            for m in range(2):
                for h, w in enumerate(_head_windows(y[56 * m:56 * m + 56], 1.0)):
                    w = pltpu.bitcast(w.astype(bf16), u32)
                    for rr in range(2):
                        pool, at = v_slot(h, 2 * p + t, rr)
                        pool[2 * n + m, at] = w[8 * rr:8 * rr + 8]
            pace.deadline(12, w)

    def project_qk(pace, n, c):
        j, t = divmod(c, 4)
        starts = [k + 112 * n + r for m in ((0, 16, 32, 48), (64, 80, 96)) for k in (D, 0) for r in m]
        rhs = _pad_rows(xn_s[c // 2][0, :D, _tile(c % 2)], 512)
        y, = pace.dots(wqk_s, (zeros_s[1], starts, slice(None), rhs))
        ks, qs = jnp.concatenate([y[:64], y[128:176]], axis=0), jnp.concatenate([y[64:128], y[176:]], axis=0)
        if c == 0:
            kmean_s[pace.zero + n] = jnp.broadcast_to(jnp.sum(ks, axis=1, keepdims=True) * (1.0 / KC), ks.shape)
        ks, qs = ks - kmean_s[n], qs * QSCALE
        k = jnp.concatenate(_head_windows(jnp.concatenate([ks[:56], ks[56:]], axis=1), 0.0), axis=0)
        kw = _words(_pad_rows(k, 128).astype(bf16).T).reshape(2, 8, 8, 128)
        for rr in reversed(range(8)):
            pool, at = k_slot(c, rr)
            pool[pl.ds(2 * n, 2), pl.ds(at, 1)] = kw[:, 7 - rr:8 - rr]
        pace.deadline(40 if c == 0 else 32, kw[1, 7])
        for m in range(2):
            for h, w in enumerate(_head_windows(qs[56 * m:56 * m + 56], 0.0)):
                qw_s[2 * n + m, h * NQ + j, pl.ds(2 * t, 2)] = _words(w.astype(bf16))
                w = w.reshape(4, 8, 128)
                for r in range(8):
                    have = [x // 8 for x in ROW_OF[h] if x % 8 == r]
                    rows = pl.ds(ROW_OF[h].index(8 * have[0] + r), len(have))
                    qb_s[2 * n + m, h * NQ + j, t // 2, rows, 0, t % 2] = jnp.broadcast_to(
                        w[have[0]:have[-1] + 1, r:r + 1], (len(have), 8, 128))
            pace.deadline(14 + 7 * m, qb_s[pace.zero, 0, 0, 0, 0, 0])

    def gather_keys(g, e):
        k = jnp.concatenate([pool[g, at] for pool, at in (k_slot(c, 7) for c in range(8 * e, 8 * e + 8))], axis=0)
        kt_s[g, e] = y = pltpu.bitcast(k, bf16).T[:2 * HP].astype(f32)
        return y

    def spread_keys(g, h, e, d):
        y = jnp.broadcast_to(kt_s[g, e, pl.ds(h * HP + ROW_OF[h][d], 1)], (128, 128)).T
        kb_s[h][KEY_AT[d][0]][KEY_AT[d][1], pl.ds(8 * e, 8)] = y.reshape(8, 2, 1, 8, 128)
        return y

    land(0)
    for chore in transpose_chores(wv_s, wqkv_v, 2 * D, 0):
        chore(None)
    pace = land(1)
    for chore in norm_x(0, pace.zero):
        chore(None)
    for p in range(6):
        if p in (1, 3):
            pace = land(2 + p // 2)
        if p == 3:
            for dst, src in ((b1_s, b1_v), (b2_s, b2_v)):
                dst[...] = jnp.broadcast_to(src[...].astype(f32).reshape(1, -1), (128, src.shape[0])).T
        pace.add(0, 36, norm_x(p + 1, pace.zero))
        project_v(pace, p)
        pace.close()
    pace = land(4)

    def spread_chore(e, d, clock):
        _gate(kt_s, pace.zero, clock)
        return clock, spread_keys(0, 0, e, d)

    for chore in transpose_chores(wqk_s, wqkv_v, 0, pace.zero, ((0, 64), (128, 192), (256, 320), (384,))):
        chore(None)
    pace.add(0, 8 * TICKS, norm_x(7, pace.zero))
    pace.add(6 * TICKS, 18 * TICKS, transpose_chores(wo_s, wo_v, 0, pace.zero))
    project_v(pace, 6)
    for n in range(4):
        if n == 1:
            pace.add(3 * TICKS, 4 * TICKS, [lambda clock, e=e: (clock, gather_keys(pace.zero, e)) for e in range(2)])
            pace.add(6 * TICKS + 7, 49 * TICKS + 7,
                     [functools.partial(spread_chore, e, d) for e in range(2) for d in range(DH)])
        for c in range(NK):
            project_qk(pace, n, c)
    project_v(pace, 7)
    pace.close()

    steps = 2 * NQ * NK

    def attend(g, carry):
        zero = zeros_s[0]
        spare = (zero, zero + 2)
        g_next, g_prev = jnp.minimum(g + 1, NP - 1), jnp.maximum(g - 1, 0)
        for e in range(2):
            gather_keys(g_next, e)
        clocks, lhs, q_words, due, stored, p_mxu = [], [], [], {}, {}, {}
        acc = partial = p_vpu = None
        for tick in range(9 * steps + 2):
            i, r = divmod(tick, 9)
            if r < 7:
                pool, at = k_slot(i % NK, r)
            else:
                pool, at = v_slot((i - 1) % steps // (NQ * NK), (i - 1) % NK, r - 7)
            for addr, v, key in due.pop(2 * tick, []) + due.pop(2 * tick + 1, []):
                pool[g, pl.ds(addr, v.shape[0])] = pltpu.bitcast(v, u32)
                stored[key] = (pool, addr)
            if (r == 5 and i > 0) or tick == 9 * steps + 1:
                p = [jnp.exp2(pltpu.bitcast(src[g, pl.ds(addr, 4)], f32)).reshape(32, 128)
                     for src, addr in (stored.pop((i - 1, a)) for a in range(2))]
                p_vpu = [jnp.concatenate([p[a][16 * x + 8 * l:16 * x + 8 * l + 8] for a in range(2) for l in range(2)],
                                         axis=1) for x in range(2)]
            if tick == 0 or (r == 5 and i + 1 < steps):
                q_words.append(qw_s[g, (i + r // 5) // NK])
            if i < steps:
                lhs.append(pool[g_prev if i == 0 and r >= 7 else g, at])
            for now in (2 * tick, 2 * tick + 1):
                clock = clocks[now - 20] if now >= 20 else None
                if 1 <= now <= 18 * steps:
                    step, (a, s) = (now - 1) // 18, divmod((now - 1) % 18, 9)
                    keys, n = kb_s[step // (NQ * NK)][s % 3], SEG_LO[s + 1] - SEG_LO[s]
                    _gate(keys, zero, clock)
                    t = keys[pl.ds(SEG_AT[s], n), step % NK] * qb_s[g, step // NK, a, pl.ds(SEG_LO[s], n)]
                    t = jnp.sum(t, axis=0).reshape(4, 8, 128)
                    partial = t if s == 0 else partial + t
                    if s == 8:
                        due[now + 2] = [(SCORES + (step % 4) * 8 + 4 * a, partial, (step, a))]
                    else:
                        due[now + 2] = [(spare[s % 2], partial[2 * (s % 2):2 * (s % 2) + 2], None)]
                h, (n, phase) = now // (9 * steps), divmod(now % (9 * steps) - 40, 18)
                if phase == 0 and 0 <= n < 2 * DH:
                    _gate(kt_s, zero, clock)
                    spread_keys(g_next if h else g, 1 - h, n // DH, n % DH)
            if r == 6:
                w = _halves(q_words[i])
                q = jnp.concatenate([w[HP * l:HP * l + HP] for l in range(4)], axis=1)
                if i >= NQ * NK:
                    q = jnp.concatenate([jnp.zeros(q.shape, bf16), q], axis=0)
                scores = _dot(pltpu.bitcast(jnp.concatenate(lhs, axis=0), bf16), _pad_rows(q, 128))
                p = jnp.exp2(scores)
                p_mxu[i] = [p[16 * x:16 * x + 16] for x in reversed(range(7))]
                clocks += [scores[8 * x:8 * x + 8, :128] for x in range(14)]
                lhs = []
            if r == 8:
                p = jnp.concatenate(p_vpu + p_mxu.pop(i - 1), axis=0) if i else tail_s[:KC]
                o = _dot(pltpu.bitcast(jnp.concatenate(lhs, axis=0), bf16), p)
                acc = o if i % NK == 1 else (acc if i else tail_s[KC:]) + o
                if i % NK == 0:
                    h, j = divmod((i - 1) % steps // NK, NQ)
                    for l in range(4):
                        o_s[4 * j + l, g if i else g_prev, h] = acc[:, 128 * l:128 * l + 128]
                clocks += [o[8 * x:8 * x + 8, :128] for x in range(4)]
                lhs = []
        for x, p in reversed(list(enumerate(p_mxu.pop(steps - 1)))):
            tail_s[pl.ds(16 * x + 16, 16)] = p
        tail_s[:16] = jnp.concatenate(p_vpu, axis=0)
        tail_s[KC:] = acc
        return carry

    lax.fori_loop(0, NP, attend, 0)

    def attend_true_max(n, carry):
        g, h, t = n // 32, (n // 16) % 2, n % 16
        q = _halves(qw_s[g, h * NQ + t // 4, pl.ds(2 * (t % 4), 2)]).astype(f32)
        r = lax.broadcasted_iota(jnp.int32, (4 * HP, 128), 0) - h * HP
        q = jnp.where((r >= 0) & (r < HP), jnp.concatenate([q] * 4, axis=0), 0.0).astype(bf16)
        k = [k_slot(c, rr) for c in range(NK) for rr in reversed(range(8))]
        scores = _dot(pltpu.bitcast(jnp.concatenate([pool[g, at] for pool, at in k], axis=0), bf16), q)
        p = jnp.exp2(scores - jnp.max(scores, axis=0, keepdims=True))
        v = [jnp.concatenate([pool[g, at] for pool, at in (v_slot(h, c, rr) for c in range(NK))], axis=1)
             for rr in range(2)]
        o_s[t, g, h] = _dot(pltpu.bitcast(jnp.concatenate(v, axis=0), bf16), p.astype(bf16))
        return carry

    land(5)

    def out_copy(j, n, l):
        return pltpu.make_async_copy(
            out_v[2 * n + l].at[j], out_hbm.at[pl.ds(HD * n, HD), pl.ds(j * BQ + 256 * l, 256)], out_sem)

    def finish(attempt):
        pace = _Pacer(zeros_s[0], 15)
        zero = pace.zero
        flag = {"unsafe": jnp.zeros((8, 128), f32)}

        def report(safe):
            for l in range(0, safe.shape[1], 128):
                flag["unsafe"] = jnp.where(safe[:, l:l + 128], flag["unsafe"], 1.0)

        def heads_chores(p):
            row = lax.broadcasted_iota(jnp.int32, (8, 256), 0)
            st = {}

            def load(g, h, r, n):
                return jnp.concatenate([o_s[2 * p + t, g, h, pl.ds(r, n)] for t in range(2)], axis=1)

            def check(first, clock):
                _gate(o_s, zero, clock)
                for g in range(4):
                    both = jnp.where(row < 4, load(first + g, 1, 0, 8), load(first + g, 0, 24, 8))
                    total = both if g == 0 else jnp.where((row & 3) == g, both, total)
                report((total >= SUM_LO) & (total <= SUM_HI))
                st["inv"] = 1.0 / total
                return st["inv"]

            def scale(g, clock):
                _gate(o_s, zero, clock)
                a, b = (load(g, h, 0, HP) * st["inv"][4 - 4 * h + g % 4:5 - 4 * h + g % 4] for h in range(2))
                y = jnp.concatenate([a[:24], jnp.where(row < 4, a[24:], b[:8]), b[8:]], axis=0)
                xn_s[p][zero, pl.ds(56 * g, 56)] = y.astype(bf16)
                for t, first in ((1, 256), (0, 320)):
                    lo, hi = max(first, 56 * g), min(first + 64, 56 * g + 56)
                    if lo < hi:
                        both = [y[lo - 56 * g:hi - 56 * g, l:l + 128] for l in (0, 128)]
                        xn_s[p][zero, pl.ds(D + lo - first, hi - lo), _tile(t)] = (both[t] - both[1 - t]).astype(bf16)
                return xn_s[p][0, pl.ds(56 * g, 8), _tile(0)]

            return [functools.partial(f, g) for first in (4, 0)
                    for f, g in [(check, first)] + [(scale, first + n) for n in range(4)]]

        def norm_h(j, zero):
            def emit(r, n, top, bottom):
                if r < 192:
                    terms = _input_terms(top[:, :256], top[:, 256:], bottom[:, :256], bottom[:, 256:])
                    hn_s[:, pl.ds(r, 8)] = jnp.stack(terms).astype(bf16)
                    for i in (0, 2, 3) if r < 128 else ():
                        t, both = int(r < 64), (terms[i][:, :128], terms[i][:, 128:])
                        hn_s[i, pl.ds(192 + r % 64, 8), _tile(t)] = (both[t] - both[1 - t]).astype(bf16)
                else:
                    for k, y in ((r, top), (r + n, bottom)):
                        s1, s2 = y[:, :256], y[:, 256:]
                        hn_s[1, pl.ds(k - 192, 8)] = s1.astype(bf16)
                        hn_s[4:, pl.ds(k - 192, 8)] = jnp.stack([s2] + [s1 + s2] * 2).astype(bf16)
                return hn_s[zero, pl.ds(0, 8), _tile(0)]
            return _norm_chores(h_s, j, pl.ds(0, BQ), ((0, 192), (384, 32)), zero, emit, report)

        def w1_chore(n, i, tile, runs, clock):
            _gate(w1_v, zero, clock)

            def load(m, r):
                return w1_v[0, pl.ds(r, 64), pl.ds(F // 2 * m + PART_LO[n], PART[n])].astype(f32)

            t = [_weight_term(i, lambda m, k: load(m, 192 * k + r)) if r < 192 else load(i % 2, r) for r in runs]
            rows = pl.ds(PART_LO[n] // 2, PART[n] // 2)
            w1_s[i, rows, tile] = pltpu.bitcast(jnp.concatenate(t, axis=0).astype(bf16).T, u32)
            return t[1], w1_s[zero + i, pl.ds(PART_LO[n] // 2, 8), tile]

        pace.add(0, 26 * TICKS,
                 [functools.partial(w1_chore, n, i, _tile(k), runs) for n in range(4) for i in range(7)
                    for k, runs in enumerate(((0, 64), (128, 64), (128, 0)) if i in (0, 2, 3) else ((0, 64), (128, 384)))])
        pace.add(11 * TICKS, 27 * TICKS, norm_h(0, zero))
        v = jnp.concatenate([pool[NP - 1, at] for pool, at in (v_slot(1, NK - 1, rr) for rr in range(2))], axis=0)
        tail = tail_s[KC:] + _dot(pltpu.bitcast(v, bf16), tail_s[:KC])

        for chore in heads_chores(0):
            chore(None)
        for p in range(NK // 2):
            if p == 1:
                for l in range(4):
                    o_s[NK - 4 + l + 4 * attempt, NP - 1, 1] = tail[:, 128 * l:128 * l + 128]
            if p + 1 < NK // 2:
                pace.add(0, 34, heads_chores(p + 1))
            for k, t, y in project(pace, wo_s, p):
                at = (p // 2, pl.ds(112 * k, 112), _tile(2 * (p % 2) + t))
                h_s[at] = x_v[at].astype(f32) + y
        pace.close()

        def ffn(j, unsafe):
            flag["unsafe"] = unsafe
            pace = _Pacer(zeros_s[0], 14)
            zero = pace.zero
            lo, size = PART_LO, PART

            def w2_chores(n):
                def chore(r, clock):
                    _gate(w2t_v, zero, clock)
                    quads = [[w2t_v[0, pl.ds(HD * m + r, 16), pl.ds(F // 2 * k + lo[n], size[n])].astype(f32)
                              for k in range(2)] for m in range(2)]
                    terms = [_weight_term(i, lambda m, k: quads[m][k]) for i in range(7)]
                    w2_s[n][:7, pl.ds(r, 16)] = jnp.stack(terms).astype(bf16)
                    return w2_s[n][zero, pl.ds(r, 8), _tile(0)]
                return [functools.partial(chore, r) for r in range(0, HD, 16)]

            def act_chore(n, r, clock):
                _gate(m_s[n % 3], zero, clock)
                m = [m_s[n % 3][i, pl.ds(r, 8)] for i in range(7)]
                us = [jnp.maximum(u, 0.0) for u in
                      (m[3] - m[4] + m[0] + m[6], m[2] + m[4], m[1] + m[3], m[2] - m[1] + m[0] + m[5])]
                acts[n // 3][:, pl.ds(lo[n] % 640 + r, 8)] = jnp.stack(_input_terms(*[u * u for u in us])).astype(bf16)
                return acts[n // 3][zero, pl.ds(lo[n] % 640 + r, 8), _tile(0)]

            pace.add(0, 100, [chore for n in (2, 0, 1, 3) for chore in w2_chores(n)])
            for n, (first, last) in enumerate(((0, 94), (0, 90), (40, 80), (0, 112))):
                def job(i, k, part=slice(None), z=0):
                    at = ((0, 0), (64, 1)) if k == 0 else ((128, k - 1), (192, k - 1))
                    rhs = jnp.concatenate([hn_s[zeros_s[z] + i, pl.ds(r, 64), _tile(t)] for r, t in at], axis=0)
                    return i, starts[part], _tile(k), rhs

                def bias(m):
                    return b1_s[pl.ds(F // 2 * m + lo[n], size[n])]

                dst, rows, starts = m_s[n % 3], pl.ds(0, size[n]), range(lo[n], lo[n] + size[n], 16)
                q = len(starts) // 4
                ys = pace.dots(w1_s, *[job(3, 0, slice(q * z, q * z + q), z) for z in range(4)])
                raw_s[0, rows] = jnp.concatenate(ys, axis=0)
                for t, i in enumerate((0, 2)):
                    y, a, b, c = pace.dots(w1_s, job(i, 0), job(i, 1), job(i, 2), job(3, 1 + t))
                    dst[i, rows] = jnp.concatenate([y + a, y + b], axis=1)
                    dst[3, rows, _tile(t)] = raw_s[zero, rows] + c
                for i in (1, 4, 5, 6):
                    y, = pace.dots(w1_s, (i, starts, pl.ds(0, 256), hn_s[zero + i]))
                    dst[i, rows] = y + jnp.concatenate([bias(i % 2) * (2.0 if i > 4 else 1.0)] * 2, axis=1)
                pace.add(first, last, [functools.partial(act_chore, n, r) for r in range(0, size[n], 8)])

            def product(k, n, i):
                rhs = acts[n // 3][zero + i, pl.ds(lo[n] % 640, size[n])]
                return pace.dots(w2_s[n], (zeros_s[1] + i, range(0, HD, 16), slice(None), rhs))[0] + sums[k][zero + i]

            def residual(n, l):
                bias = jnp.concatenate([b2_s[pl.ds(HD * n, HD)]] * 2, axis=1)
                return h_s[j, pl.ds(HD * n, HD), pl.ds(256 * l, 256)] + bias

            def emit(n, l, y):
                out_v[2 * n + l][j] = y.astype(bf16)
                out_copy(j, n, l).start()

            for i in ORDER:
                parts = [pl.ds(0, HD)] if i != ORDER[-1] else [pl.ds(0, HD // 2), pl.ds(HD // 2, HD // 2)]
                for k, rows in enumerate(parts):
                    sums[0][i, rows] = _dot(w2_s[2][zeros_s[1] + i, rows],
                                            acts[0][zeros_s[k] + i, pl.ds(lo[2], 128)])
            pace.add(8 * TICKS, 15 * TICKS, norm_h(jnp.minimum(j + 1, NQ - 1), zero))
            for k in range(2):
                for i in ORDER:
                    sums[1 - k][i] = product(k, k, i)
            keep[0][0] = product(0, 3, 1)
            pace.close()
            keep[1][0] = y = product(0, 3, 3)
            emit(1, 0, y + keep[0][zero] + residual(1, 0))
            keep[1][1] = y = product(0, 3, 2)
            keep[1][2] = y - keep[0][zero] + residual(1, 1)
            y = product(0, 3, 4)
            emit(0, 1, y + keep[1][zero + 1] + residual(0, 1))
            keep[0][1] = keep[1][zero] - y + residual(0, 0)
            keep[0][2] = product(0, 3, 0)
            emit(0, 0, keep[0][zero + 1] + keep[0][zero + 2] + product(0, 3, 6))
            emit(1, 1, keep[1][zero + 2] + keep[0][zero + 2] + product(0, 3, 5))
            return flag["unsafe"]

        unsafe = lax.fori_loop(0, NQ, ffn, flag["unsafe"])
        redo = (jnp.max(unsafe) > 0.0) & (attempt == 0)

        @pl.when(redo)
        def _():
            lax.fori_loop(0, H * S // 128, attend_true_max, 0)

        for j in range(NQ):
            for n in range(4):
                out_copy(j, n // 2, n % 2).wait()
        return jnp.where(redo, 1, 2)

    lax.while_loop(lambda attempt: attempt < 2, finish, 0)


@jax.jit
def pallas_sequential_preLN__softmax_full_mha__dense_activation_squared_relu__prompt_kernel(
    A_x: jax.Array,
    A_wqkv: jax.Array,
    A_wo: jax.Array,
    B_x: jax.Array,
    B_w1: jax.Array,
    B_b1: jax.Array,
    B_w2: jax.Array,
    B_b2: jax.Array,
):
    del B_x
    in_hbm = pl.BlockSpec(memory_space=pl.ANY)
    out_t = pl.pallas_call(
        _kernel,
        out_shape=jax.ShapeDtypeStruct((D, S), bf16),
        in_specs=[in_hbm] * 7,
        out_specs=in_hbm,
        scratch_shapes=[
            pltpu.VMEM((NQ + 1, D, BQ), bf16),
            pltpu.VMEM((2, D, 3 * D), bf16),
            pltpu.VMEM((2, D, D), bf16),
            pltpu.VMEM((2, D, F), bf16),
            pltpu.VMEM((2, D, F), bf16),
            pltpu.VMEM((2, D, 512), u32),
            pltpu.VMEM((2, HD, 640), u32),
            pltpu.VMEM((2, HD, 640), u32),
            pltpu.VMEM((8, F // 4, 384), u32),
            [pltpu.VMEM((8, HD, n), bf16) for n in PART],
            pltpu.VMEM((D, 128), f32),
            [pltpu.VMEM((2, 512, 256), bf16)] * (2 * NQ),
            pltpu.VMEM((2, 256, 128), f32),
            [pltpu.VMEM((8, 256, 256), f32)] * 3,
            [pltpu.VMEM((3, HD, 256), f32)] * 2,
            [pltpu.VMEM((7, HD, 256), f32)] * 2,
            [pltpu.VMEM((7, n, 256), bf16) for n in (640, 256)],
            pltpu.VMEM((7, 256, 256), bf16),
            pltpu.VMEM((NQ + 1, D, BQ), f32),
            [pltpu.VMEM((NP, PIECES + 6 * NK, 8, 128), u32)] * 2,
            pltpu.VMEM((NP, 2 * NQ, 8, 8, 128), u32),
            pltpu.VMEM((NP, 2 * NQ, 2, DH, 1, 2, 8, 128), f32),
            pltpu.VMEM((4, 112, 128), f32),
            pltpu.VMEM((NP + 1, 2, 2 * HP, 128), f32),
            [[pltpu.VMEM((12, NK + 1, 2, 1, 8, 128), f32)] * 3] * 2,
            pltpu.VMEM((KC + HP, BQ), f32),
            pltpu.VMEM((NK + 4, NP, 2, HP, 128), f32),
            [pltpu.VMEM((NQ, HD, 256), bf16)] * 4,
            pltpu.VMEM((F, 128), f32),
            pltpu.VMEM((F,), bf16),
            pltpu.VMEM((D,), bf16),
            pltpu.SMEM((4,), jnp.int32),
            pltpu.SemaphoreType.DMA((6,)),
            pltpu.SemaphoreType.DMA(()),
        ],
        compiler_params=pltpu.CompilerParams(vmem_limit_bytes=112 * 2**20, disable_bounds_checks=True),
        name="fused_block",
    )(A_x.reshape(S, D).T, A_wqkv, A_wo, B_w1, B_b1, B_w2.T, B_b2)
    return out_t.T.reshape(1, S, D)
```

```python
import functools
import math

import jax
import jax.numpy as jnp
from jax import lax
import jax.experimental.pallas as pl
import jax.experimental.pallas.tpu as pltpu

S, D, H, DH, F = 2048, 448, 16, 28, 1792
BQ = 512
NQ = S // BQ
KC = 128
NK = S // KC
HP = 32
NP = H // 2
HD = D // 2
EPS = 1e-5
QSCALE = DH ** -0.5 * math.log2(math.e)
SUM_LO, SUM_HI = 2.0 ** -20, 2.0 ** 100
bf16, f32, u32 = jnp.bfloat16, jnp.float32, jnp.uint32

SCORES, PIECES = 8, 40

SEG_LO = [-(-(DH * s) // 9) for s in range(10)]
SEG_AT = [sum(SEG_LO[t + 1] - SEG_LO[t] for t in range(s % 3, s, 3)) for s in range(9)]
KEY_AT = [(s % 3, SEG_AT[s] + d - SEG_LO[s]) for s in range(9) for d in range(SEG_LO[s], SEG_LO[s + 1])]
ROW_PAIRS = [[(8 * k + r, 8 * k + r + 16) for r in range(8) for k in range(2) if (k, r // 4) != (1 - h, 1 - h)]
             + [(12 + 4 * h + r, 14 + 4 * h + r) for r in range(2)] for h in range(2)]

PASS_ROWS = ((384, 256), (0, 64), (128, 192), (384, 320), (256, 320))

ORDER = (1, 3, 2, 4, 0, 6, 5)
PART_LO, PART = (0, 256, 512, 640), (256, 256, 128, 256)
TICKS = HD // 16


def _dot(a, b):
    return jnp.dot(a, b, preferred_element_type=f32)


def _tile(t):
    return pl.ds(128 * t, 128)


def _pad_rows(x, n):
    return jnp.concatenate([x, jnp.zeros((n - x.shape[0], x.shape[1]), x.dtype)], axis=0)


def _words(x):
    return pltpu.bitcast(x, u32).reshape(x.shape[0] // 16, 8, 128)


def _halves(w):
    return pltpu.bitcast(w.reshape(w.shape[0] * 8, 128), bf16)


def _head_windows(y, fill):
    low = lax.broadcasted_iota(jnp.int32, (8, y.shape[1]), 0) < 4
    return (jnp.concatenate([y[:24], jnp.where(low, y[24:32], fill)], axis=0),
            jnp.concatenate([jnp.where(low, fill, y[24:32]), y[32:]], axis=0))


def _weight_term(i, quad):
    a, sign, b = (((0, 0), 1, (1, 1)), ((1, 0), 1, (1, 1)), ((0, 0), 0, None), ((1, 1), 0, None),
                  ((0, 0), 1, (0, 1)), ((1, 0), -1, (0, 0)), ((0, 1), -1, (1, 1)))[i]
    return quad(*a) if sign == 0 else quad(*a) + quad(*b) if sign > 0 else quad(*a) - quad(*b)


def _input_terms(b11, b12, b21, b22):
    return [b11 + b22, b11, b12 - b22, b21 - b11, b22, b11 + b12, b21 + b22]


def _retype(v, dtype):
    if v.dtype == dtype:
        return v
    if v.dtype != f32:
        v = v.astype(f32) if v.dtype == bf16 else pltpu.bitcast(v, f32)
    return v if dtype == f32 else v.astype(bf16) if dtype == bf16 else pltpu.bitcast(v, dtype)


def _gate(ref, zero, value, row=0):
    if value is not None:
        at = (zero + (ref.shape[0] - 1), *(0,) * (len(ref.shape) - 3), pl.ds(row, 8), _tile(0))
        ref[at] = _retype(value, ref.dtype)


class _Pacer:
    def __init__(self, zero, delay):
        self.zero, self.delay = zero, delay
        self.tick, self.todo, self.due = 0, {}, {}

    def add(self, first, last, chores):
        for n, chore in enumerate(chores):
            self.todo.setdefault(self.tick + first + n * (last - first) // len(chores), []).append(chore)

    def deadline(self, ticks, v):
        self.due.setdefault(self.tick + ticks, []).extend(v[-8:, l:l + 128] for l in range(0, v.shape[1], 128))

    def dots(self, w_ref, *jobs):
        pieces, ticks = [[] for _ in jobs], len(jobs[0][1])
        for n in range(ticks):
            for k, v in enumerate(self.due.pop(self.tick + n, [])):
                _gate(w_ref, self.zero, v, 8 * k)
            for got, (i, starts, cols, _) in zip(pieces, jobs):
                r = starts[n]
                got.append(w_ref[i, pl.ds(r, 16) if w_ref.dtype == bf16 else pl.ds(r // 2, 8), cols])
        lhs = [jnp.concatenate(got, axis=0) for got in pieces]
        ys = [_dot(a if a.dtype == bf16 else pltpu.bitcast(a, bf16), job[3]) for a, job in zip(lhs, jobs)]
        for n in range(ticks):
            for chore in self.todo.pop(self.tick + n, []):
                done = chore(ys[0][16 * n:16 * n + 8, :128])
                for k, v in enumerate(done if isinstance(done, tuple) else (done,)):
                    self.deadline(max(n + self.delay + 28 * k, ticks), v)
        self.tick += ticks
        return ys

    def dot_pair(self, w_ref, i, rows, x):
        firsts = [range(r, r + 112, 16) for r in rows]
        for k, first in enumerate(firsts):
            shared, y = self.dots(
                w_ref, (i, first, _tile(4), jnp.concatenate([x(256, 64, 0), x(320, 64, 1)], axis=0)),
                (i, first, pl.ds(128, 384), jnp.concatenate([x(0, 256, 0), x(384, 128, 0)], axis=0)))
            yield k, 0, shared + y
            if k == 0:
                late = shared
                continue
            rhs = [x(384, 128, 1), x(0, 128, 1), x(128, 128, 1)]
            part, y = self.dots(w_ref, (i, firsts[0], _tile(k - 1), rhs[k - 1]),
                                (i, first, pl.ds(0, 384), jnp.concatenate(rhs, axis=0)))
            late = late + part
            yield k, 1, shared + y
        yield 0, 1, late

    def close(self):
        assert not self.todo


def _norm_chores(src, j, cols, runs, zero, emit, report=None):
    step = 8 * BQ // cols.size
    st = {}

    def load(r, n):
        return src[j, pl.ds(r, n), cols].astype(f32)

    def total(r, clock):
        _gate(src, zero, clock)
        y = jnp.sum(load(r, 4 * step).reshape(-1, 8, cols.size), axis=0)
        st["acc"] = y if r == 0 else st["acc"] + y
        return st["acc"]

    def spread(r, clock):
        _gate(src, zero, clock)
        if r == 0:
            st["mean"] = jnp.sum(st["acc"], axis=0, keepdims=True) * (1.0 / D)
        y = load(r, 4 * step) - st["mean"]
        y = jnp.sum((y * y).reshape(-1, 8, cols.size), axis=0)
        st["acc"] = y if r == 0 else st["acc"] + y
        return st["acc"]

    def scale(r, n, clock):
        _gate(src, zero, clock)
        if r == 0:
            var = jnp.sum(st["acc"], axis=0, keepdims=True) * (1.0 / D)
            st["inv"] = lax.rsqrt(var + EPS)
            if report:
                report(var < jnp.inf)
        return emit(r, n, *((load(k, step) - st["mean"]) * st["inv"] for k in (r, r + n)))

    return ([functools.partial(f, r) for f in (total, spread) for r in range(0, D, 4 * step)]
            + [functools.partial(scale, r, n) for first, n in runs for r in range(first, first + n, step)])


def _kernel(x_hbm, wqkv_hbm, wo_hbm, w1_hbm, b1_hbm, w2t_hbm, b2_hbm, out_hbm,
            x_v, wqkv_v, wo_v, w1_v, w2t_v,
            wqk_s, wv_s, wo_s, w1_s, w2_s, b2_s, xn_s, raw_s, m_s, keep, sums, acts, hn_s, h_s,
            pools, qw_s, qb_s, kmean_s, kt_s, kb_s, tail_s, o_s, out_v,
            b1_s, b1_v, b2_v, zeros_s, in_sems, out_sem):
    waves = [[(wqkv_hbm.at[:, pl.ds(2 * D, D)], wqkv_v.at[0, :, pl.ds(2 * D, D)])]]
    waves += [[(x_hbm.at[:, pl.ds(j * BQ, BQ)], x_v.at[j]) for j in js] for js in ((0,), (1,), (2, 3))]
    waves += [[(wqkv_hbm.at[:, pl.ds(0, 2 * D)], wqkv_v.at[0, :, pl.ds(0, 2 * D)]), (wo_hbm, wo_v.at[0])],
              [(w1_hbm, w1_v.at[0]), (w2t_hbm, w2t_v.at[0])]]
    waves[2] += [(b1_hbm, b1_v), (b2_hbm, b2_v)]
    waves = [[pltpu.make_async_copy(src, dst, in_sems.at[i]) for src, dst in wave] for i, wave in enumerate(waves)]

    def land(i):
        for copy in waves[i]:
            copy.wait()
        for k in ((2,), (3, 4), (), (), (5,), ())[i]:
            for copy in waves[k]:
                copy.start()
        return _Pacer(zeros_s[0], 16)

    for copy in waves[0] + waves[1]:
        copy.start()
    for z in range(4):
        zeros_s[z] = 0
    tail_s[...] = jnp.zeros(tail_s.shape, f32)

    def k_slot(c, rr):
        return pools[(c + rr) % 2], PIECES + c * 4 + rr // 2

    def v_slot(h, c, rr):
        return pools[(c + rr) % 2], h * NK + (PIECES + 4 * NK + c)

    def norm_x(p, zero):
        def emit(r, n, top, bottom):
            xn_s[p][zero, pl.ds(r, 16)] = top.astype(bf16)
            xn_s[p][zero, pl.ds(r + n, 16)] = bottom.astype(bf16)
            if 256 <= r < 320:
                diff = jnp.concatenate([bottom[:, :128] - bottom[:, 128:], top[:, 128:] - top[:, :128]], axis=1)
                xn_s[p][zero, pl.ds(D + r - 256, 16)] = diff.astype(bf16)
            return xn_s[p][0, pl.ds(r, 8), _tile(0)]
        return _norm_chores(x_v, p // 2, pl.ds(256 * (p % 2), 256), ((0, 128), (256, 64), (384, 32)), zero, emit)

    def transpose_chores(dst, src, first, zero):
        def chore(k, c, clock):
            _gate(src, zero, clock)
            n = min(256, 2 * dst.shape[1] - c)
            y = jnp.concatenate([src[0, pl.ds(r, 64), pl.ds(first + c, n)] for r in PASS_ROWS[k]], axis=0)
            y = pltpu.bitcast(y.T, u32)
            dst[0, pl.ds(c // 2, n // 2), _tile(k)] = y
            return clock, y
        return [functools.partial(chore, k, c) for c in range(0, 2 * dst.shape[1], 256) for k in range(5)]

    def project(pace, w_ref, p, rows=range(0, D, 112)):
        return pace.dot_pair(w_ref, zeros_s[1], rows, lambda r, n, t: xn_s[p][0, pl.ds(r, n), _tile(t)])

    def project_v(pace, p):
        for n, t, y in project(pace, wv_s, p):
            for m in range(2):
                for h, w in enumerate(_head_windows(y[56 * m:56 * m + 56], 1.0)):
                    w = pltpu.bitcast(w.astype(bf16), u32)
                    for rr in range(2):
                        pool, at = v_slot(h, 2 * p + t, rr)
                        pool[2 * n + m, at] = w[8 * rr:8 * rr + 8]
            pace.deadline(12, w)

    def put_keys(pace, n, c, ks):
        if c == 0:
            kmean_s[pace.zero + n] = jnp.broadcast_to(jnp.sum(ks, axis=1, keepdims=True) * (1.0 / KC), ks.shape)
        ks = ks - kmean_s[n]
        k = jnp.concatenate(_head_windows(jnp.concatenate([ks[:56], ks[56:]], axis=1), 0.0), axis=0)
        kw = _words(_pad_rows(k, 128).astype(bf16).T).reshape(2, 8, 8, 128)
        for rr in reversed(range(8)):
            pool, at = k_slot(c, rr)
            pool[pl.ds(2 * n, 2), pl.ds(at, 1)] = kw[:, 7 - rr:8 - rr]
        pace.deadline(46 + 10 * (c < 2), kw[1, 7])

    def put_queries(pace, n, c, qs, late):
        j, t = divmod(c, 4)
        low = lax.broadcasted_iota(jnp.int32, (DH // 2, 8, 128), 1) < 4
        for m in range(2):
            for h, w in enumerate(_head_windows(qs[56 * m:56 * m + 56] * QSCALE, 0.0)):
                qw_s[2 * n + m, h * NQ + j, pl.ds(2 * t, 2)] = _words(w.astype(bf16))
                lo, hi = (jnp.stack([jnp.broadcast_to(w[r:r + 1], (8, 128)) for r in rows])
                          for rows in zip(*ROW_PAIRS[h]))
                qb_s[2 * n + m, h * NQ + j, t // 2, :, 0, t % 2] = jnp.where(low, lo, hi)
            pace.deadline(10 + late + 5 * m, qb_s[pace.zero, 0, 0, 0, 0, 0])

    def project_qk(pace, half, p):
        for k, t, y in project(pace, wqk_s, p, [HD * half + r for r in (0, D, 112, D + 112)]):
            if k % 2:
                put_keys(pace, 2 * half + k // 2, 2 * p + t, y)
            else:
                put_queries(pace, 2 * half + k // 2, 2 * p + t, y, 3 * (t == k // 2))

    def gather_keys(g, e):
        k = jnp.concatenate([pool[g, at] for pool, at in (k_slot(c, 7) for c in range(8 * e, 8 * e + 8))], axis=0)
        kt_s[g, e, 1] = y = pltpu.bitcast(k, bf16).T[:2 * HP].astype(f32)
        low = (lax.broadcasted_iota(jnp.int32, y.shape, 1) & 4) == 0
        kt_s[g, e, 0] = jnp.where(low, pltpu.roll(y, 124, 1), pltpu.roll(y, 4, 1))
        return y

    def spread_keys(g, h, e, d):
        lo, hi = (kt_s[g, e, d // 14, pl.ds(h * HP + r, 1)] for r in ROW_PAIRS[h][d % 14])
        low = (lax.broadcasted_iota(jnp.int32, (1, 128), 1) & 4) == 0
        y = jnp.broadcast_to(jnp.where(low, lo, hi), (128, 128)).T
        kb_s[h][KEY_AT[d][0]][KEY_AT[d][1], pl.ds(8 * e, 8)] = y.reshape(8, 2, 1, 8, 128)
        return y

    land(0)
    for chore in transpose_chores(wv_s, wqkv_v, 2 * D, 0):
        chore(None)
    pace = land(1)
    for chore in norm_x(0, pace.zero):
        chore(None)
    for p in range(5):
        if p in (1, 3):
            pace = land(2 + p // 2)
        if p == 3:
            for dst, src in ((b1_s, b1_v), (b2_s, b2_v)):
                dst[...] = jnp.broadcast_to(src[...].astype(f32).reshape(1, -1), (128, src.shape[0])).T
        pace.add(0, 36, norm_x(p + 1, pace.zero))
        project_v(pace, p)
        pace.close()
    pace = land(4)

    def spread_chore(e, d, clock):
        _gate(kt_s, pace.zero, clock)
        return clock, spread_keys(0, 0, e, d)

    for chore in transpose_chores(wqk_s, wqkv_v, 0, pace.zero):
        chore(None)
    pace.add(0, 36, norm_x(6, pace.zero))
    project_v(pace, 5)
    pace.add(0, 8 * TICKS, norm_x(7, pace.zero))
    pace.add(6 * TICKS, 18 * TICKS, transpose_chores(wo_s, wo_v, 0, pace.zero))
    project_v(pace, 6)
    for n in range(NK):
        if n in (5, 10):
            pace.add(0, 1, [lambda clock, e=n // 10: (clock, gather_keys(pace.zero, e))])
            pace.add(50, 240 if n == 5 else 305, [functools.partial(spread_chore, n // 10, d) for d in range(DH)])
        project_qk(pace, n // 8, n % 8)
    project_v(pace, 7)
    pace.close()

    steps = 2 * NQ * NK

    def attend(g, carry):
        zero = zeros_s[0]
        spare, g_again = (zero, zero + 2), g + zero
        g_next, g_prev = jnp.minimum(g + 1, NP - 1), jnp.maximum(g - 1, 0)
        for e in range(2):
            gather_keys(g_next, e)
        clocks, lhs, q_words, due, stored, p_mxu = [], [], [], {}, {}, {}
        acc = partial = p_vpu = None
        for tick in range(9 * steps + 2):
            i, r = divmod(tick, 9)
            if r < 7:
                pool, at = k_slot(i % NK, r)
            else:
                pool, at = v_slot((i - 1) % steps // (NQ * NK), (i - 1) % NK, r - 7)
            for addr, v, key in due.pop(2 * tick, []) + due.pop(2 * tick + 1, []):
                pool[g, pl.ds(addr, v.shape[0])] = pltpu.bitcast(v, u32)
                stored[key] = (pool, addr)
            if (r == 5 and i > 0) or tick == 9 * steps + 1:
                p = [jnp.exp2(pltpu.bitcast(src[g, pl.ds(addr, 4)], f32)).reshape(32, 128)
                     for src, addr in (stored.pop((i - 1, a)) for a in range(2))]
                p_vpu = [jnp.concatenate([p[a][16 * x + 8 * l:16 * x + 8 * l + 8] for a in range(2) for l in range(2)],
                                         axis=1) for x in range(2)]
            if tick == 0 or (r == 5 and i + 1 < steps):
                q_words.append(qw_s[g, (i + r // 5) // NK])
            if i < steps:
                lhs.append(pool[g_prev if i == 0 and r >= 7 else g, at])
            for now in (2 * tick, 2 * tick + 1):
                clock = clocks[now - 20] if now >= 20 else None
                if 0 <= now - 1 < 18 * steps:
                    step, (a, s) = (now - 1) // 18, divmod((now - 1) % 18, 9)
                    keys, lo, hi = kb_s[step // (NQ * NK)][s % 3], SEG_LO[s], SEG_LO[s + 1]
                    _gate(keys, zero, clock)
                    for d, e in ((lo, 14), (14, hi)) if lo < 14 < hi else ((lo, hi),):
                        t = (keys[pl.ds(SEG_AT[s] + d - lo, e - d), step % NK]
                             * qb_s[g if d < 14 else g_again, step // NK, a, pl.ds(d % 14, e - d)])
                        t = jnp.sum(t, axis=0).reshape(4, 8, 128)
                        partial = t if d == 0 else (pltpu.roll(partial, 4, 1) if d == 14 else partial) + t
                    if s == 8:
                        due[now + 2] = [(SCORES + (step % 4) * 8 + 4 * a, partial, (step, a))]
                    else:
                        due[now + 2] = [(spare[s % 2], partial[2 * (s % 2):2 * (s % 2) + 2], None)]
                h, (n, phase) = now // (9 * steps), divmod(now % (9 * steps) - 58, 18)
                if phase == 0 and 0 <= n < 2 * DH:
                    _gate(kt_s, zero, clock)
                    spread_keys(g_next if h else g, 1 - h, n // DH, n % DH)
            if r == 6:
                w = _halves(q_words[i])
                q = jnp.concatenate([w[HP * l:HP * l + HP] for l in range(4)], axis=1)
                if i >= NQ * NK:
                    q = jnp.concatenate([jnp.zeros(q.shape, bf16), q], axis=0)
                scores = _dot(pltpu.bitcast(jnp.concatenate(lhs, axis=0), bf16), _pad_rows(q, 128))
                p = jnp.exp2(scores)
                p_mxu[i] = [p[16 * x:16 * x + 16] for x in reversed(range(7))]
                clocks += [scores[8 * x:8 * x + 8, :128] for x in range(14)]
                lhs = []
            if r == 8:
                p = jnp.concatenate(p_vpu + p_mxu.pop(i - 1), axis=0) if i else tail_s[:KC]
                o = _dot(pltpu.bitcast(jnp.concatenate(lhs, axis=0), bf16), p)
                acc = o if i % NK == 1 else (acc if i else tail_s[KC:]) + o
                if i % NK == 0:
                    h, j = divmod((i - 1) % steps // NK, NQ)
                    for l in range(4):
                        o_s[4 * j + l, g if i else g_prev, h] = acc[:, 128 * l:128 * l + 128]
                clocks += [o[8 * x:8 * x + 8, :128] for x in range(4)]
                lhs = []
        for x, p in reversed(list(enumerate(p_mxu.pop(steps - 1)))):
            tail_s[pl.ds(16 * x + 16, 16)] = p
        tail_s[:16] = jnp.concatenate(p_vpu, axis=0)
        tail_s[KC:] = acc
        return carry

    lax.fori_loop(0, NP, attend, 0)

    def attend_true_max(n, carry):
        g, h, t = n // 32, (n // 16) % 2, n % 16
        q = _halves(qw_s[g, h * NQ + t // 4, pl.ds(2 * (t % 4), 2)]).astype(f32)
        r = lax.broadcasted_iota(jnp.int32, (4 * HP, 128), 0) - h * HP
        q = jnp.where((r >= 0) & (r < HP), jnp.concatenate([q] * 4, axis=0), 0.0).astype(bf16)
        k = [k_slot(c, rr) for c in range(NK) for rr in reversed(range(8))]
        scores = _dot(pltpu.bitcast(jnp.concatenate([pool[g, at] for pool, at in k], axis=0), bf16), q)
        p = jnp.exp2(scores - jnp.max(scores, axis=0, keepdims=True))
        v = [jnp.concatenate([pool[g, at] for pool, at in (v_slot(h, c, rr) for c in range(NK))], axis=1)
             for rr in range(2)]
        o_s[t, g, h] = _dot(pltpu.bitcast(jnp.concatenate(v, axis=0), bf16), p.astype(bf16))
        return carry

    land(5)

    def out_copy(j, n, l):
        return pltpu.make_async_copy(
            out_v[2 * n + l].at[j], out_hbm.at[pl.ds(HD * n, HD), pl.ds(j * BQ + 256 * l, 256)], out_sem)

    def finish(attempt):
        pace = _Pacer(zeros_s[0], 15)
        zero = pace.zero
        flag = {"unsafe": jnp.zeros((8, 128), f32)}

        def report(safe):
            for l in range(0, safe.shape[1], 128):
                flag["unsafe"] = jnp.where(safe[:, l:l + 128], flag["unsafe"], 1.0)

        def heads_chores(p):
            row = lax.broadcasted_iota(jnp.int32, (8, 256), 0)
            st = {}

            def load(g, h, r, n):
                return jnp.concatenate([o_s[2 * p + t, g, h, pl.ds(r, n)] for t in range(2)], axis=1)

            def check(first, clock):
                _gate(o_s, zero, clock)
                for g in range(4):
                    both = jnp.where(row < 4, load(first + g, 1, 0, 8), load(first + g, 0, 24, 8))
                    total = both if g == 0 else jnp.where((row & 3) == g, both, total)
                report((total >= SUM_LO) & (total <= SUM_HI))
                st["inv"] = 1.0 / total
                return st["inv"]

            def scale(g, clock):
                _gate(o_s, zero, clock)
                a, b = (load(g, h, 0, HP) * st["inv"][4 - 4 * h + g % 4:5 - 4 * h + g % 4] for h in range(2))
                y = jnp.concatenate([a[:24], jnp.where(row < 4, a[24:], b[:8]), b[8:]], axis=0)
                xn_s[p][zero, pl.ds(56 * g, 56)] = y.astype(bf16)
                for t, first in ((1, 256), (0, 320)):
                    lo, hi = max(first, 56 * g), min(first + 64, 56 * g + 56)
                    if lo < hi:
                        both = [y[lo - 56 * g:hi - 56 * g, l:l + 128] for l in (0, 128)]
                        xn_s[p][zero, pl.ds(D + lo - first, hi - lo), _tile(t)] = (both[t] - both[1 - t]).astype(bf16)
                return xn_s[p][0, pl.ds(56 * g, 8), _tile(0)]

            return [functools.partial(f, g) for first in (4, 0)
                    for f, g in [(check, first)] + [(scale, first + n) for n in range(4)]]

        def norm_h(j, zero):
            def emit(r, n, top, bottom):
                if r < 192:
                    terms = _input_terms(top[:, :256], top[:, 256:], bottom[:, :256], bottom[:, 256:])
                    hn_s[:, pl.ds(r, 8)] = jnp.stack(terms).astype(bf16)
                    for i in (0, 2, 3) if r < 128 else ():
                        t, both = int(r < 64), (terms[i][:, :128], terms[i][:, 128:])
                        hn_s[i, pl.ds(192 + r % 64, 8), _tile(t)] = (both[t] - both[1 - t]).astype(bf16)
                else:
                    for k, y in ((r, top), (r + n, bottom)):
                        s1, s2 = y[:, :256], y[:, 256:]
                        hn_s[1, pl.ds(k - 192, 8)] = s1.astype(bf16)
                        hn_s[4:, pl.ds(k - 192, 8)] = jnp.stack([s2] + [s1 + s2] * 2).astype(bf16)
                return hn_s[zero, pl.ds(0, 8), _tile(0)]
            return _norm_chores(h_s, j, pl.ds(0, BQ), ((0, 192), (384, 32)), zero, emit, report)

        def w1_chore(n, i, tile, runs, clock):
            _gate(w1_v, zero, clock)

            def load(m, r):
                return w1_v[0, pl.ds(r, 64), pl.ds(F // 2 * m + PART_LO[n], PART[n])].astype(f32)

            t = [_weight_term(i, lambda m, k: load(m, 192 * k + r)) if r < 192 else load(i % 2, r) for r in runs]
            rows = pl.ds(PART_LO[n] // 2, PART[n] // 2)
            w1_s[i, rows, tile] = pltpu.bitcast(jnp.concatenate(t, axis=0).astype(bf16).T, u32)
            return t[1], w1_s[zero + i, pl.ds(PART_LO[n] // 2, 8), tile]

        w1_passes = [((0, 64), (128, 64), (128, 0)) if i in (0, 2, 3) else ((0, 64), (128, 384)) for i in range(7)]
        pace.add(0, 26 * TICKS, [functools.partial(w1_chore, n, i, _tile(k), runs)
                                 for n in range(4) for i in range(7) for k, runs in enumerate(w1_passes[i])])
        pace.add(11 * TICKS, 27 * TICKS, norm_h(0, zero))
        v = jnp.concatenate([pool[NP - 1, at] for pool, at in (v_slot(1, NK - 1, rr) for rr in range(2))], axis=0)
        tail = tail_s[KC:] + _dot(pltpu.bitcast(v, bf16), tail_s[:KC])

        for chore in heads_chores(0):
            chore(None)
        for p in range(NK // 2):
            if p == 1:
                for l in range(4):
                    o_s[NK - 4 + l + 4 * attempt, NP - 1, 1] = tail[:, 128 * l:128 * l + 128]
            if p + 1 < NK // 2:
                pace.add(0, 34, heads_chores(p + 1))
            for k, t, y in project(pace, wo_s, p):
                at = (p // 2, pl.ds(112 * k, 112), _tile(2 * (p % 2) + t))
                h_s[at] = x_v[at].astype(f32) + y
        pace.close()

        def ffn(j, unsafe):
            flag["unsafe"] = unsafe
            pace = _Pacer(zeros_s[0], 14)
            zero = pace.zero
            lo, size = PART_LO, PART

            def w2_chores(n):
                def chore(r, clock):
                    _gate(w2t_v, zero, clock)
                    quads = [[w2t_v[0, pl.ds(HD * m + r, 16), pl.ds(F // 2 * k + lo[n], size[n])].astype(f32)
                              for k in range(2)] for m in range(2)]
                    terms = [_weight_term(i, lambda m, k: quads[m][k]) for i in range(7)]
                    w2_s[n][:7, pl.ds(r, 16)] = jnp.stack(terms).astype(bf16)
                    return w2_s[n][zero, pl.ds(r, 8), _tile(0)]
                return [functools.partial(chore, r) for r in range(0, HD, 16)]

            def act_chore(n, r, clock):
                _gate(m_s[n % 3], zero, clock)
                m = [m_s[n % 3][i, pl.ds(r, 8)] for i in range(7)]
                us = [jnp.maximum(u, 0.0) for u in
                      (m[3] - m[4] + m[0] + m[6], m[2] + m[4], m[1] + m[3], m[2] - m[1] + m[0] + m[5])]
                acts[n // 3][:, pl.ds(lo[n] % 640 + r, 8)] = jnp.stack(_input_terms(*[u * u for u in us])).astype(bf16)
                return acts[n // 3][zero, pl.ds(lo[n] % 640 + r, 8), _tile(0)]

            pace.add(0, 100, [chore for n in (2, 0, 1, 3) for chore in w2_chores(n)])
            for n, (first, last) in enumerate(((0, 94), (0, 90), (40, 80), (0, 112))):
                def job(i, k, part=slice(None), z=0):
                    at = ((0, 0), (64, 1)) if k == 0 else ((128, k - 1), (192, k - 1))
                    rhs = jnp.concatenate([hn_s[zeros_s[z] + i, pl.ds(r, 64), _tile(t)] for r, t in at], axis=0)
                    return i, starts[part], _tile(k), rhs

                def bias(m):
                    return b1_s[pl.ds(F // 2 * m + lo[n], size[n])]

                dst, rows, starts = m_s[n % 3], pl.ds(0, size[n]), range(lo[n], lo[n] + size[n], 16)
                q = len(starts) // 4
                ys = pace.dots(w1_s, *[job(3, 0, slice(q * z, q * z + q), z) for z in range(4)])
                raw_s[0, rows] = jnp.concatenate(ys, axis=0)
                for t, i in enumerate((0, 2)):
                    y, a, b, c = pace.dots(w1_s, job(i, 0), job(i, 1), job(i, 2), job(3, 1 + t))
                    dst[i, rows] = jnp.concatenate([y + a, y + b], axis=1)
                    dst[3, rows, _tile(t)] = raw_s[zero, rows] + c
                for i in (1, 4, 5, 6):
                    y, = pace.dots(w1_s, (i, starts, pl.ds(0, 256), hn_s[zero + i]))
                    dst[i, rows] = y + jnp.concatenate([bias(i % 2) * (2.0 if i > 4 else 1.0)] * 2, axis=1)
                pace.add(first, last, [functools.partial(act_chore, n, r) for r in range(0, size[n], 8)])

            def product(k, n, i):
                rhs = acts[n // 3][zero + i, pl.ds(lo[n] % 640, size[n])]
                return pace.dots(w2_s[n], (zeros_s[1] + i, range(0, HD, 16), slice(None), rhs))[0] + sums[k][zero + i]

            def residual(n, l):
                bias = jnp.concatenate([b2_s[pl.ds(HD * n, HD)]] * 2, axis=1)
                return h_s[j, pl.ds(HD * n, HD), pl.ds(256 * l, 256)] + bias

            def emit(n, l, y):
                out_v[2 * n + l][j] = y.astype(bf16)
                out_copy(j, n, l).start()

            for i in ORDER:
                parts = [pl.ds(0, HD)] if i != ORDER[-1] else [pl.ds(0, HD // 2), pl.ds(HD // 2, HD // 2)]
                for k, rows in enumerate(parts):
                    sums[0][i, rows] = _dot(w2_s[2][zeros_s[1] + i, rows],
                                            acts[0][zeros_s[k] + i, pl.ds(lo[2], 128)])
            pace.add(8 * TICKS, 15 * TICKS, norm_h(jnp.minimum(j + 1, NQ - 1), zero))
            for k in range(2):
                for i in ORDER:
                    sums[1 - k][i] = product(k, k, i)
            keep[0][0] = product(0, 3, 1)
            pace.close()
            keep[1][0] = y = product(0, 3, 3)
            emit(1, 0, y + keep[0][zero] + residual(1, 0))
            keep[1][1] = y = product(0, 3, 2)
            keep[1][2] = y - keep[0][zero] + residual(1, 1)
            y = product(0, 3, 4)
            emit(0, 1, y + keep[1][zero + 1] + residual(0, 1))
            keep[0][1] = keep[1][zero] - y + residual(0, 0)
            keep[0][2] = product(0, 3, 0)
            emit(0, 0, keep[0][zero + 1] + keep[0][zero + 2] + product(0, 3, 6))
            emit(1, 1, keep[1][zero + 2] + keep[0][zero + 2] + product(0, 3, 5))
            return flag["unsafe"]

        unsafe = lax.fori_loop(0, NQ, ffn, flag["unsafe"])
        redo = (jnp.max(unsafe) > 0.0) & (attempt == 0)

        @pl.when(redo)
        def _():
            lax.fori_loop(0, H * S // 128, attend_true_max, 0)

        for j in range(NQ):
            for n in range(4):
                out_copy(j, n // 2, n % 2).wait()
        return jnp.where(redo, 1, 2)

    lax.while_loop(lambda attempt: attempt < 2, finish, 0)


@jax.jit
def pallas_sequential_preLN__softmax_full_mha__dense_activation_squared_relu__prompt_kernel(
    A_x: jax.Array,
    A_wqkv: jax.Array,
    A_wo: jax.Array,
    B_x: jax.Array,
    B_w1: jax.Array,
    B_b1: jax.Array,
    B_w2: jax.Array,
    B_b2: jax.Array,
):
    del B_x
    in_hbm = pl.BlockSpec(memory_space=pl.ANY)
    out_t = pl.pallas_call(
        _kernel,
        out_shape=jax.ShapeDtypeStruct((D, S), bf16),
        in_specs=[in_hbm] * 7,
        out_specs=in_hbm,
        scratch_shapes=[
            pltpu.VMEM((NQ + 1, D, BQ), bf16),
            pltpu.VMEM((2, D, 3 * D), bf16),
            pltpu.VMEM((2, D, D), bf16),
            pltpu.VMEM((2, D, F), bf16),
            pltpu.VMEM((2, D, F), bf16),
            pltpu.VMEM((2, D, 640), u32),
            pltpu.VMEM((2, HD, 640), u32),
            pltpu.VMEM((2, HD, 640), u32),
            pltpu.VMEM((8, F // 4, 384), u32),
            [pltpu.VMEM((8, HD, n), bf16) for n in PART],
            pltpu.VMEM((D, 128), f32),
            [pltpu.VMEM((2, 512, 256), bf16)] * (2 * NQ),
            pltpu.VMEM((2, 256, 128), f32),
            [pltpu.VMEM((8, 256, 256), f32)] * 3,
            [pltpu.VMEM((3, HD, 256), f32)] * 2,
            [pltpu.VMEM((7, HD, 256), f32)] * 2,
            [pltpu.VMEM((7, n, 256), bf16) for n in (640, 256)],
            pltpu.VMEM((7, 256, 256), bf16),
            pltpu.VMEM((NQ + 1, D, BQ), f32),
            [pltpu.VMEM((NP, PIECES + 6 * NK, 8, 128), u32)] * 2,
            pltpu.VMEM((NP, 2 * NQ, 8, 8, 128), u32),
            pltpu.VMEM((NP, 2 * NQ, 2, DH // 2, 1, 2, 8, 128), f32),
            pltpu.VMEM((4, 112, 128), f32),
            pltpu.VMEM((NP + 1, 2, 2, 2 * HP, 128), f32),
            [[pltpu.VMEM((12, NK + 1, 2, 1, 8, 128), f32)] * 3] * 2,
            pltpu.VMEM((KC + HP, BQ), f32),
            pltpu.VMEM((NK + 4, NP, 2, HP, 128), f32),
            [pltpu.VMEM((NQ, HD, 256), bf16)] * 4,
            pltpu.VMEM((F, 128), f32),
            pltpu.VMEM((F,), bf16),
            pltpu.VMEM((D,), bf16),
            pltpu.SMEM((4,), jnp.int32),
            pltpu.SemaphoreType.DMA((6,)),
            pltpu.SemaphoreType.DMA(()),
        ],
        compiler_params=pltpu.CompilerParams(vmem_limit_bytes=112 * 2**20, disable_bounds_checks=True),
        name="fused_block",
    )(A_x.reshape(S, D).T, A_wqkv, A_wo, B_w1, B_b1, B_w2.T, B_b2)
    return out_t.T.reshape(1, S, D)
```
